```python
import jax
import jax.numpy as jnp

def _softmax(x, axis=-1):
    return jax.nn.softmax(x, axis=axis)
def _gelu(x):
    return jax.nn.gelu(x, approximate=True)
def _silu(x):
    return jax.nn.silu(x)
def _sigmoid(x):
    return jax.nn.sigmoid(x)
def _layernorm(x, axis=-1, eps=1e-5):
    m = jnp.mean(x, axis=axis, keepdims=True)
    v = jnp.var(x, axis=axis, keepdims=True)
    return (x - m) / jnp.sqrt(v + eps)
def _scatter_add(tgt, idx, src, axis=0):
    return tgt.at[idx].add(src)
def _segment_sum(src, seg, n):
    return jax.ops.segment_sum(src, seg, n)
class _Rng:
    def __init__(self, key):
        self._k = key
    def _next(self):
        self._k, sub = jax.random.split(self._k)
        return sub
    def normal(self, shape):
        return jax.random.normal(self._next(), shape, dtype=jnp.bfloat16)
    def randint(self, lo, hi, shape):
        return jax.random.randint(self._next(), shape, lo, hi, dtype=jnp.int32)
    def uniform(self, shape, lo=0.0, hi=1.0):
        return jax.random.uniform(self._next(), shape, jnp.bfloat16, lo, hi)
    def permutation(self, n):
        return jax.random.permutation(self._next(), n)


kernel_name = 'recurrent_scan__linear_kernel_hedgehog__moe_arch_mod__prompt'

def setup_inputs():
    _rng = _Rng(jax.random.key(int.from_bytes(__import__("os").urandom(4), "little")))
    _w = (lambda a: (lambda t: t.astype(jnp.bfloat16) if jnp.issubdtype(t.dtype, jnp.floating) else t)(jnp.asarray(a)))
    def _A_setup():
        B, S, D, H = 1, 2048, 1024, 32
        Dh = D // H
        return {
            "x": _w((lambda *s: _rng.normal(s) * 0.05)(B, S, D)),
            "wqkv": _w((lambda *s: _rng.normal(s) * 0.05)(D, 3 * D)),
            "w_phi": _w((lambda *s: _rng.normal(s) * 0.05)(H, Dh, Dh) * (Dh ** -0.5)),
            "wo": _w((lambda *s: _rng.normal(s) * 0.05)(D, D)),
        }
    _A_in = _A_setup()

    def _B_setup():
        B, S, D, F, C = 1, 2048, 1024, 3584, 1
        return {
            "x": _w((lambda *s: _rng.normal(s) * 0.05)(B, S, D)),
            "w_r": _w((lambda *s: _rng.normal(s) * 0.05)(D)),
            "w_gate": _w((lambda *s: _rng.normal(s) * 0.05)(D, F)),
            "w_up": _w((lambda *s: _rng.normal(s) * 0.05)(D, F)),
            "w_down": _w((lambda *s: _rng.normal(s) * 0.05)(F, D)),
        }
    _B_in = _B_setup()

    return {
        "A_x": _A_in["x"],
        "A_wqkv": _A_in["wqkv"],
        "A_w_phi": _A_in["w_phi"],
        "A_wo": _A_in["wo"],
        "B_x": _B_in["x"],
        "B_w_r": _B_in["w_r"],
        "B_w_gate": _B_in["w_gate"],
        "B_w_up": _B_in["w_up"],
        "B_w_down": _B_in["w_down"],
    }

def reference(A_x, A_wqkv, A_w_phi, A_wo, B_x, B_w_r, B_w_gate, B_w_up, B_w_down):
    def _A_ref(x, wqkv, w_phi, wo):
        B, S, D = x.shape
        H = 32; Dh = D // H
        qkv = (lambda x, *d: x.transpose(*d))((x @ wqkv).reshape(B, S, 3, H, Dh), 2, 0, 3, 1, 4)
        q, k, v = qkv[0], qkv[1], qkv[2]
        pq = jnp.einsum("bhsd,hdf->bhsf", q, w_phi)
        pk = jnp.einsum("bhsd,hdf->bhsf", k, w_phi)
        phi_q = jnp.concatenate([_softmax(pq, axis=-1), _softmax(-pq, axis=-1)], axis=-1)
        phi_k = jnp.concatenate([_softmax(pk, axis=-1), _softmax(-pk, axis=-1)], axis=-1)
        kv = jnp.einsum("bhsf,bhsd->bhfd", phi_k, v)
        z  = jnp.einsum("bhsf->bhf", phi_k)
        num = jnp.einsum("bhqf,bhfd->bhqd", phi_q, kv)
        den = jnp.einsum("bhqf,bhf->bhq", phi_q, z)[..., None] + 1e-6
        o = num / den
        return (lambda x, *d: x.transpose(*d))(o, 0, 2, 1, 3).reshape(B, S, D) @ wo

    def _B_ref(x, w_r, w_gate, w_up, w_down):
        B, S, D = x.shape
        C = 1
        r = x @ w_r
        idx = jnp.argsort(-r, axis=-1)[:, :C]
        idx_e = jnp.repeat(idx.reshape(B, C, 1), D, axis=2)
        x_sel = jnp.take_along_axis(x, idx_e, axis=1)
        g = _silu(x_sel @ w_gate)
        u = x_sel @ w_up
        y = (g * u) @ w_down
        r_sel = _sigmoid(jnp.take_along_axis(r, idx, axis=1))
        y = y * r_sel.reshape(B, C, 1)
        b_off = (jnp.arange(B) * S).reshape(B, 1)
        flat_idx = (idx + b_off).reshape(B * C)
        zero = (x * 0.0).reshape(B * S, D)
        upd = _scatter_add(zero, flat_idx, y.reshape(B * C, D), axis=0)
        return x + upd.reshape(B, S, D)

    x = A_x
    xn = _layernorm(x, axis=-1)
    s = _A_ref(xn, A_wqkv, A_w_phi, A_wo)
    g = _silu(_B_ref(xn, B_w_r, B_w_gate, B_w_up, B_w_down))
    return x + s * g
```

```python
import contextlib
import functools

import jax
import jax.numpy as jnp
from jax import lax
import jax.experimental.pallas as pl
import jax.experimental.pallas.tpu as pltpu

F32 = jnp.float32
BF16 = jnp.bfloat16
U32 = jnp.uint32
LOG2E = 1.4426950408889634
NT = (((1,), (1,)), ((), ()))

S, D, H, DH, FF = 2048, 1024, 32, 32, 3584
NP = H // 2
PR = 2 * DH
NU = 4
UW = D // NU
FC = 256
T = 256
HT = T // 2
HD = D // 2
NTILE = S // T


def _bf16_round(v):
    return v.astype(BF16).astype(F32)


def _pack(even, odd):
    return pltpu.bitcast(pltpu.pack_elementwise([even, odd], packed_dtype=BF16), U32)


def _rows(words):
    return pltpu.bitcast(words, BF16)


def _allreduce(r, op):
    r = op(r, pltpu.roll(r, 4, 0))
    return op(r, pltpu.roll(r, 2, 0))


def _dual_exp(p):
    p3 = p.reshape(8, 8, p.shape[1])
    mx = _allreduce(jnp.max(p3, axis=0), jnp.maximum)
    mn = _allreduce(jnp.min(p3, axis=0), jnp.minimum)
    ep = jnp.exp2(p3 - mx[None])
    en = jnp.exp2(mn[None] - p3)
    rp = pl.reciprocal(_allreduce(jnp.sum(ep, axis=0), jnp.add), approx=True)
    rn = pl.reciprocal(_allreduce(jnp.sum(en, axis=0), jnp.add), approx=True)
    return ep, en, rp, rn


def _lhs_term(k, a11, a12, a21, a22):
    return (lambda: a11() + a22(), lambda: a21() + a22(), a11, a22, lambda: a11() + a12(),
            lambda: a21() - a11(), lambda: a12() - a22())[k]()


def _rhs_term(k, b11, b12, b21, b22):
    return (lambda: b11() + b22(), b11, lambda: b12() - b22(), lambda: b21() - b11(), b22,
            lambda: b11() + b12(), lambda: b21() + b22())[k]()


def _quadrant(m, r, c):
    if (r, c) == (0, 0):
        return m(0) + m(3) - m(4) + m(6)
    if (r, c) == (0, 1):
        return m(2) + m(4)
    if (r, c) == (1, 0):
        return m(1) + m(3)
    return m(0) - m(1) + m(2) + m(5)


def _better(a, b):
    take = (b[0] > a[0]) | ((b[0] == a[0]) & (b[1] < a[1]))
    return jnp.where(take, b[0], a[0]), jnp.where(take, b[1], a[1])


def _zero_after(v):
    return jnp.where(v > jnp.inf, 1.0, 0.0)


def _touch(words):
    tiles = [w[r:r + 8, c:c + 128] for w in words for r in range(0, w.shape[0], 8) for c in range(0, w.shape[1], 128)]
    return pltpu.bitcast(functools.reduce(jnp.bitwise_or, tiles), F32)


def _held(v, zero):
    if zero is None:
        return v
    z = jnp.tile(pltpu.bitcast(zero, U32), (v.shape[0] // 8, v.shape[1] // 128))
    return pltpu.bitcast(pltpu.bitcast(v, U32) | z, F32)


def _spread(tasks, nslots):
    return [tasks[s * len(tasks) // nslots:(s + 1) * len(tasks) // nslots] for s in range(nslots)]


def _merge(*lists):
    keyed = [((k + 0.5) / len(l), n, t) for n, l in enumerate(lists) for k, t in enumerate(l)]
    return [t for _, _, t in sorted(keyed, key=lambda e: e[:2])]


def _kernel(x_hbm, wqkv_hbm, wphi_hbm, wo_hbm, wr_hbm, wg_hbm, wu_hbm, wd_hbm, out_hbm,
            x_v, w_v, wphi_v, wr_v, wo_v, wg_v, wu_v, wd_v, out_v, fix_v,
            staged, pin_f, pin_u, x_sem, w_sem, misc_sem, out_sem, pin_sem, *, cfg):
    scope = lambda n: jax.named_scope(n) if (cfg['scopes'] == 1 or (cfg['scopes'] == 2 and n.startswith('w_'))) else contextlib.nullcontext()

    def x_copy(i):
        rows = pl.ds(i * T, T)
        return pltpu.make_async_copy(x_hbm.at[rows], x_v.at[rows], x_sem.at[i])

    def w_copy(m, u):
        cols = pl.ds(m * D + u * UW, UW)
        return pltpu.make_async_copy(wqkv_hbm.at[:, cols], w_v.at[:, cols], w_sem.at[m, u])

    wphi_cp = pltpu.make_async_copy(wphi_hbm, wphi_v, misc_sem.at[0])
    wr_cp = pltpu.make_async_copy(wr_hbm, wr_v, misc_sem.at[1])
    wo_cp = pltpu.make_async_copy(wo_hbm, wo_v, misc_sem.at[2])
    wg_cp = pltpu.make_async_copy(wg_hbm, wg_v, misc_sem.at[3])
    wu_cp = pltpu.make_async_copy(wu_hbm, wu_v, misc_sem.at[4])
    wd_cp = pltpu.make_async_copy(wd_hbm, wd_v, misc_sem.at[5])

    nghost = [0]

    def ghost(v):
        k = nghost[0]
        nghost[0] += 1
        st['sink'][k] = v
        st['sink'][k] = jnp.zeros((8, 128), F32)
        return st['sink'][k]

    due = []

    def gate_of(kind, gate):
        return gate if kind in cfg['gates'].split() else None

    def run(tasks, gate=None):
        for t in tasks:
            done = t(gate)
            if done is not None and cfg['slack'][done[0]]:
                due.append([cfg['slack'][done[0]], ghost(done[1])])

    def products(slot, lhs, rhs, dims, tasks, jobs, placed=False):
        for k, group in enumerate(tasks if placed else _spread(tasks, 7)):
            words = lhs(k)
            for d in due:
                d[0] -= 1
            ready = [d[1] for d in due if d[0] <= 0]
            due[:] = [d for d in due if d[0] > 0]
            if ready:
                z = pltpu.bitcast(functools.reduce(jnp.add, ready), U32)
                last = jnp.concatenate([words[-8:, :-128], words[-8:, -128:] | z], axis=1)
                words = jnp.concatenate([words[:-8], last], axis=0)
            res = lax.dot_general(_rows(words), _rows(rhs(k)), dims, preferred_element_type=F32)
            m_v[slot][k] = res
            if cfg['mdl']:
                due.append([cfg['mdl'], ghost(_touch([pltpu.bitcast(res, U32)]))])
            if group:
                run(group, ghost(res[0:8]))
            if k == 6 and cfg['fence']:
                m_v[slot][7 + zero, 0:8, :] = res[0:8]
            for job in jobs.get(k, ()):
                job()

    def prep_bd():
        r_i = lax.broadcasted_iota(jnp.int32, (128, DH), 0)
        c_i = lax.broadcasted_iota(jnp.int32, (128, DH), 1)
        sel = ((r_i % DH) == c_i).astype(BF16)
        rep = lax.dot_general(sel, wphi_v[...], NT, preferred_element_type=F32)
        r_i = lax.broadcasted_iota(jnp.int32, (128, D), 0)
        c_i = lax.broadcasted_iota(jnp.int32, (128, D), 1)
        bd_v[...] = jnp.where((r_i // DH) == ((c_i % 128) // DH), rep, 0.0).astype(BF16)

    def fold(m, u, slot):
        for g in range(2):
            c0 = u * UW + g * 128
            t = lax.dot_general(bd_v[:, c0:c0 + 128], w_v[:, m * D + c0:m * D + c0 + 128], NT,
                                preferred_element_type=F32)
            for c in range(8):
                fold_ref(slot, g, c)[...] = t[:, c * 128:(c + 1) * 128]

    def fold_ref(slot, g, c):
        k = g * 8 + c
        return ot_v.at[k // 4, k % 4]

    def fold_terms(m, u, slot, c, q, gate):
        rows = slice(q * PR, (q + 1) * PR)
        a = [_held(fold_ref(slot, g, h * 4 + c)[rows, :], gate_of('fq', gate)) * LOG2E for g in range(2) for h in range(2)]
        outs = []
        for k in range(7):
            t = _lhs_term(k, *[(lambda v=v: v) for v in a])
            outs.append(_pack(t[:DH], t[DH:]))
            wt_v[m][u, k, q * DH:(q + 1) * DH, c * 128:(c + 1) * 128] = outs[-1]
        return 'fq' if m == 0 else 'fk', _touch(outs)

    def v_terms(u, c, ks, gate):
        c0 = 2 * D + u * UW
        blk = lambda g, h: (lambda: _held(w_v[h * HD + c * 128:h * HD + (c + 1) * 128,
                                        c0 + g * 128:c0 + (g + 1) * 128].astype(F32), gate_of('fv', gate)))
        outs = []
        for k in ks:
            t = _lhs_term(k, blk(0, 0), blk(0, 1), blk(1, 0), blk(1, 1))
            outs.append(pltpu.bitcast(t.astype(BF16).T, U32))
            wt_v[2][u, k, :, c * 128:(c + 1) * 128] = outs[-1]
        return 'fv', _touch(outs)

    def wo_terms(u, g, q, gate):
        b = [wo_v[g * UW + r * 128 + q * PR:g * UW + r * 128 + (q + 1) * PR,
                  u * UW + c * 128:u * UW + (c + 1) * 128].astype(F32) for r in range(2) for c in range(2)]
        b = [_held(v, gate_of('wo', gate)) for v in b]
        outs = []
        for k in range(7):
            t = _rhs_term(k, *[(lambda v=v: v) for v in b])
            outs.append(_pack(t[:DH], t[DH:]))
            wos_v[u, k, g * PR + q * DH:g * PR + (q + 1) * DH, :] = outs[-1]
        return 'wo', _touch(outs)

    def fold_tasks(m, u):
        return [functools.partial(fold_terms, m, u, 0, c, q) for c in range(4) for q in range(2)]

    def v_tasks_of(u):
        return [functools.partial(v_terms, u, c, ks) for ks in ((0, 1, 2), (3, 4), (5, 6)) for c in range(4)]

    def ln_rows(xf, gate=None):
        mean = jnp.sum(xf, axis=1, keepdims=True) * (1.0 / D)
        if gate is not None and cfg['gin']:
            mean = mean + gate[:, 0:1]
        cen = xf - mean
        var = jnp.sum(cen * cen, axis=1, keepdims=True) * (1.0 / D)
        den = _bf16_round(jnp.sqrt(_bf16_round(_bf16_round(var) + 1e-5)))
        return (xf - _bf16_round(mean)) * pl.reciprocal(den, approx=True)

    def ln_norm(i, c, half, e, gate):
        r0 = i * T + half * HT + c * 16
        words = pltpu.bitcast(x_v[r0:r0 + 16, :], U32)
        xf = pltpu.unpack_elementwise(words, index=e, packed_dtype=BF16, unpacked_dtype=F32)
        xn = ln_rows(_held(xf, gate_of('ln', gate)))
        xf_v[c % 4, half, e] = xn
        return 'ln', _touch([pltpu.bitcast(xn, U32)])

    def ln_route(i, c, gate):
        top = None
        outs = []
        wr = wr_rows if gate is None else wr_rows + jnp.tile(gate, (1, 8))
        for half in range(2):
            r0 = i * T + half * HT + c * 16
            outs.append(_pack(xf_v[c % 4, half, 0], xf_v[c % 4, half, 1]))
            xn_v[r0 // 2:r0 // 2 + 8, :] = outs[-1]
            for e in range(2):
                r = _bf16_round(jnp.sum(xf_v[c % 4, half, e] * wr, axis=1, keepdims=True))
                r = jnp.broadcast_to(r, (8, 128))
                tok = 2 * lax.broadcasted_iota(jnp.int32, (8, 128), 0) + (r0 + e)
                if top is None:
                    top = (jnp.where(r != r, -jnp.inf, r), jnp.where(r != r, S, tok))
                else:
                    top = _better(top, (r, tok))
        best_v[i * 8 + c], bidx_v[i * 8 + c] = top
        return 'ln', _touch(outs + [pltpu.bitcast(t, U32) for t in top])

    def ln_terms(i, c, ks, gate):
        outs = []
        for k in ks:
            blk = lambda half, e, h: (lambda: _held(xf_v[c % 4, half, e, :, h * HD:(h + 1) * HD], gate_of('lt', gate)))
            t = [_rhs_term(k, blk(0, e, 0), blk(1, e, 0), blk(0, e, 1), blk(1, e, 1)) for e in range(2)]
            outs.append(_pack(*t))
            xs_v[i % 2][i // 2, k, c * 8:(c + 1) * 8, :] = outs[-1]
        return 'lt', _touch(outs)

    def ln_tasks(i):
        first = lambda c: [P(ln_norm, i, c, half, e) for half in range(2) for e in range(2)]
        second = lambda c: [P(ln_terms, i, c, (0, 1, 2)), P(ln_terms, i, c, (3, 4, 5, 6)), P(ln_route, i, c)]
        tasks = first(0)
        for c in range(1, 8):
            tasks += _merge(first(c), second(c - 1))
        return tasks + second(7)

    def proj(m, u, i, slot, tasks, jobs={}, placed=False):
        products(slot, lambda k: wt_v[m][u, k], lambda k: xs_v[i % 2][i // 2, k], NT, tasks, jobs, placed)

    def pair_block(slot, q, t):
        rows = slice((q % 2) * PR, (q % 2 + 1) * PR)
        return _quadrant(lambda k: m_v[slot][k, rows, :], q // 2, t)

    def phi_k(i, u, slot, q, t, gate):
        p = u * 4 + q
        ep, en, rp, rn = _dual_exp(_held(pair_block(slot, q, t), gate_of('phi', gate)))
        php = (ep * rp[None]).reshape(PR, 128)
        phn = (en * rn[None]).reshape(PR, 128)
        words = _pack(php, phn)
        phi_v[u][q, :, t * 128:(t + 1) * 128] = words
        z = jnp.concatenate([php, phn], axis=0)
        if i or t:
            z = z + z_v[p]
        z_v[p] = z
        return 'phi', _touch([words, pltpu.bitcast(z, U32)])

    def v_pack(u, slot, q, gate):
        outs = []
        for t in range(2):
            vt = _held(pair_block(slot, q, t), gate_of('vp', gate))
            outs.append(_pack(vt[:DH], vt[DH:]))
            vt_v[q, :, t * 128:(t + 1) * 128] = outs[-1]
        return 'vp', _touch(outs)

    def kv_update(i, u, qs):
        for q in qs:
            upd = lax.dot_general(_rows(vt_v[q]), _rows(phi_v[u][q]), NT, preferred_element_type=F32)
            if i:
                upd = upd + kv_v[u * 4 + q]
            kv_v[u * 4 + q] = upd
            due.append([3, ghost(_touch([pltpu.bitcast(upd, U32)]))])

    def kv_finish(p, gate):
        r_i = lax.broadcasted_iota(jnp.int32, (PR, 128), 0)
        c_i = lax.broadcasted_iota(jnp.int32, (PR, 128), 1)
        zb = jnp.broadcast_to(jnp.sum(_held(z_v[p], gate_of('kf', gate)), axis=1, keepdims=True), (128, 128))
        z_v[p] = zb
        kvt_v[p] = jnp.where((r_i % 2) == ((c_i // 2) % 2), kv_v[p], 0.0).astype(BF16)
        return 'kf', _touch([pltpu.bitcast(zb, U32)])

    P = functools.partial
    nothing = lambda gate: None

    wr_cp.start()
    x_copy(0).start()
    wr_cp.wait()
    wphi_cp.start()
    w_copy(1, 0).start()
    wr8 = wr_v[...].astype(F32)
    zero = jnp.where(wr8 > jnp.inf, 1, 0)[0, 0]
    wr_rows = jnp.concatenate([jnp.broadcast_to(wr8[c:c + 1], (8, 128)) for c in range(8)], axis=1)
    st = {k: r.at[zero] if (cfg['dyn'] == 'all' or k.rstrip('0123') in cfg['dyn'].split()) else r.at[0] for k, r in staged.items()}
    bd_v, wos_v, xn_v, vt_v, ot_v, kv_v, kvt_v, z_v, best_v, bidx_v, xb_v, hb_v, gu_v, y_v, sfix_v = [
        st[k] for k in 'bd wos xn vt ot kv kvt z best bidx xb hb gu y sfix'.split()]
    wt_v = [st['wt%d' % m] for m in range(3)]
    xs_v = [st['xs0'], st['xs1']]
    m_v = [st['m%d' % m] for m in range(4)]
    phi_v = [st['phi%d' % m] for m in range(4)]
    os_v = [st['os0'], st['os1']]
    xf_v = st['xf']
    with scope('w_x0'):
        x_copy(0).wait()
    first = ln_tasks(0)
    for t in first[:len(first) // 2]:
        t(None)
    w_copy(1, 1).start()
    with scope('w_wphi'):
        wphi_cp.wait()
    prep_bd()
    for t in first[len(first) // 2:]:
        t(None)
    w_copy(1, 2).start()
    with scope('w_k0'):
        w_copy(1, 0).wait()
    fold(1, 0, 0)
    for t in fold_tasks(1, 0):
        t(None)

    def softmax_k(i, u, slot):
        return [P(phi_k, i, u, slot, q, t) for q in (2, 0, 3, 1) for t in range(2)]

    def pack_v(u, slot):
        return [P(v_pack, u, slot, q) for q in (2, 3, 0, 1)]

    def sync(starts, waits, name):
        def job():
            for cp in starts:
                cp.start()
            with scope(name):
                for cp in waits:
                    cp.wait()
        return job

    with scope('p1_0'):
        fa, va = cfg['fold_at'], cfg['v_at']
        after = [w_copy(1, 3), w_copy(2, 0), w_copy(2, 1), x_copy(1)]
        for u in range(NU):
            tasks = softmax_k(0, u - 1, 2 + (u - 1) % 2) if u else []
            if u < NU - 1:
                job = [sync([after[u]], [w_copy(1, u + 1)], 'w_k%d' % (u + 1)), P(fold, 1, u + 1, 0)]
                late = _spread(fold_tasks(1, u + 1), 6 - fa)
                proj(1, u, 0, 2 + u % 2, _spread(tasks, fa + 1) + late, {fa: job}, True)
            else:
                job = [sync([after[u]], [w_copy(2, 0)], 'w_v0')]
                proj(1, u, 0, 2 + u % 2, _spread(tasks, va + 1) + _spread(v_tasks_of(0), 6 - va), {va: job}, True)
        after = [[w_copy(2, 2)], [w_copy(2, 3)], [x_copy(2)]]
        need = [[w_copy(2, 1)], [x_copy(1), w_copy(2, 2)], [w_copy(2, 3)]]
        ln = ln_tasks(1) + [nothing] * cfg['ln_pad']
        ln = [[]] * (7 + va + 1) + _spread(ln, 21 - va - 1)
        for u in range(NU):
            tasks = softmax_k(0, NU - 1, 3) if u == 0 else pack_v(u - 1, (u - 1) % 2)
            jobs = {6: [P(kv_update, 0, u - 1, (2, 3, 0, 1))]} if u else {}
            if u + 1 < NU:
                jobs[va] = [sync(after[u], need[u], 'w_v%d' % (u + 1))]
                tasks = _spread(tasks, va + 1) + _spread(v_tasks_of(u + 1), 6 - va)
            else:
                tasks = _spread(tasks, 7)
            proj(2, u, 0, u % 2, [a + b for a, b in zip(tasks, ln[7 * u:7 * u + 7])], jobs, True)

    prev = (0, NU - 1)
    wo_tasks = [P(wo_terms, u, g, q) for u in range(NU) for g in range(4) for q in range(2)]
    for i in range(1, NTILE):
      with scope('p1_%d' % i):
        if i == 1:
            sync([x_copy(t) for t in range(3, NTILE)] + [w_copy(0, u) for u in range(NU)], [x_copy(2)], 'w_x2')()
        if i == 2:
            sync([wo_cp], [x_copy(t) for t in range(3, NTILE)], 'w_x3')()
        if i == 3:
            sync([wg_cp, wu_cp, wd_cp],
                 [w_copy(0, u) for u in range(NU)] + [wo_cp], 'w_q')()
        for u in range(NU):
            k_tasks = pack_v(prev[1], 1)
            v_tasks = softmax_k(i, u, 0)
            jobs = [{}, {}]
            for pos, qs in cfg['kv_at']:
                jobs[pos // 7][pos % 7] = [P(kv_update, *prev, qs)]
            if i + 1 < NTILE:
                ln = _spread(ln_tasks(i + 1) + [nothing] * cfg['ln_pad'], NU)[u]
                nk = len(ln) * cfg['ln_k'] // 14
                k_tasks = _merge(k_tasks, ln[:nk])
                v_tasks = _merge(v_tasks, ln[nk:])
            else:
                k_tasks = _merge(k_tasks, wo_tasks[8 + 6 * u:12 + 6 * u])
                v_tasks = _merge(v_tasks, wo_tasks[12 + 6 * u:14 + 6 * u])
                if u > 1:
                    k_tasks = _merge(k_tasks, [P(kv_finish, (u - 2) * 4 + q) for q in range(4)])
            if 3 <= i < 7 and u % 2:
                k_tasks = _merge(k_tasks, wo_tasks[(i - 3) * 2 + u // 2:(i - 3) * 2 + u // 2 + 1])
            if 3 <= i < 3 + NU:
                if u == 0:
                    jobs[0][0] = [P(fold, 0, i - 3, 0)]
                v_tasks = _merge(v_tasks, fold_tasks(0, i - 3)[2 * u:2 * u + 2])
            proj(1, u, i, 0, k_tasks, jobs[0])
            proj(2, u, i, 1, v_tasks, jobs[1])
            prev = (i, u)

    best = jnp.max(jnp.max(best_v[...], axis=0), axis=0, keepdims=True)
    bidx = jnp.min(jnp.min(jnp.where(best_v[...] == best[None], bidx_v[...], S), axis=0), axis=0, keepdims=True)
    idx_raw = bidx[0, 0]
    idx = jnp.where(idx_raw == S, 0, idx_raw)
    gate_r = _bf16_round(jax.nn.sigmoid(jnp.where(bidx == S, jnp.nan, best)))[:, 0:1]
    row16 = lax.broadcasted_iota(jnp.int32, (16, D), 0)
    grp = idx // 16
    fix_grp = jnp.where(idx >= S - T, 0, grp)

    def ffn_input(gate):
        xb_v[...] = ln_rows(x_v[pl.ds(pl.multiple_of(grp * 16, 16), 16), :].astype(F32)).astype(BF16)
        sfix_v[...] = jnp.zeros(sfix_v.shape, F32)

    def ffn_up(c, which, h):
        gu_v[c % 2, which, h] = jnp.dot(xb_v[:, h * HD:(h + 1) * HD],
                                        (wg_v, wu_v)[which][h * HD:(h + 1) * HD, c * 128:(c + 1) * 128],
                                        preferred_element_type=F32)
        if (which, h) == (1, 1):
            g = gu_v[c % 2, 0, 0] + gu_v[c % 2, 0, 1]
            hb_v[c % 2] = (g * jax.nn.sigmoid(g) * (gu_v[c % 2, 1, 0] + gu_v[c % 2, 1, 1])).astype(BF16)

    def ffn_down(c, h):
        part = jnp.dot(hb_v[c % 2], wd_v[c * 128:(c + 1) * 128, h * HD:(h + 1) * HD], preferred_element_type=F32)
        if c:
            part = part + y_v[:, h * HD:(h + 1) * HD]
        y_v[:, h * HD:(h + 1) * HD] = part
        due.append([3, ghost(_touch([pltpu.bitcast(part, U32)]))])

    ffn = []
    for c in range(FF // 128):
        ffn += [P(ffn_up, c, which, h) for which in range(2) for h in range(2)]
        if c:
            ffn += [P(ffn_down, c - 1, h) for h in range(2)]
    ffn += [P(ffn_down, FF // 128 - 1, h) for h in range(2)]

    def phi_q(u, slot, q, t, gate):
        p = u * 4 + q
        ep, en, rp, rn = _dual_exp(_held(pair_block(slot, q, t), gate_of('phi', gate)))
        a = jnp.sum(ep * z_v[p, :PR].reshape(8, 8, 128), axis=0)
        b = jnp.sum(en * z_v[p, PR:].reshape(8, 8, 128), axis=0)
        rd = pl.reciprocal(_allreduce(rp * a + rn * b, jnp.add) + 1e-6, approx=True)
        words = _pack((ep * (rp * rd)[None]).reshape(PR, 128), (en * (rn * rd)[None]).reshape(PR, 128))
        phi_v[u][q, :, t * 128:(t + 1) * 128] = words
        return 'phi', _touch([words])

    def attend(u, qs=(2, 3, 0, 1)):
        for q in qs:
            o = jnp.dot(kvt_v[u * 4 + q], _rows(phi_v[u][q]), preferred_element_type=F32)
            for t in range(2):
                ot_v[q // 2, t, (q % 2) * PR:(q % 2 + 1) * PR, :] = o[:, t * 128:(t + 1) * 128]

    def o_terms(j, u, ks, gate):
        blk = lambda t, g: (lambda: _held(ot_v[g, t], gate_of('ot', gate)))
        outs = []
        for k in ks:
            term = _lhs_term(k, blk(0, 0), blk(0, 1), blk(1, 0), blk(1, 1))
            outs.append(pltpu.bitcast(term.astype(BF16).T, U32))
            os_v[j % 2][k, :, u * 128:(u + 1) * 128] = outs[-1]
        return 'ot', _touch(outs)

    def out_proj(j, u, slot, tasks, jobs={}):
        products(slot, lambda k: os_v[j % 2][k], lambda k: wos_v[u, k],
                 (((1,), (0,)), ((), ())), tasks, jobs)

    def routed_update(cols):
        y = y_v[:, cols]
        mine = lax.broadcasted_iota(jnp.int32, y.shape, 0) == idx % 16
        yrow = jnp.sum(jnp.where(mine, y, 0.0), axis=0, keepdims=True)
        return _bf16_round(_bf16_round(yrow) * gate_r)

    def gated(xf, b, s):
        return xf + s * (b * pl.reciprocal(1.0 + jnp.exp2(b * (-LOG2E)), approx=True))

    def epilogue(j, u, slot, t, c, gate):
        nr = 64
        r0 = j * T + t * HT + c * nr
        cols = slice(u * UW, (u + 1) * UW)
        s = jnp.concatenate([_quadrant(lambda k: m_v[slot][k, c * nr:(c + 1) * nr, :], t, h) for h in range(2)],
                            axis=1)
        b = _held(_rows(xn_v[r0 // 2:(r0 + nr) // 2, cols]).astype(F32), gate_of('epi', gate))
        s = _held(s, gate_of('epi', gate))
        extra = []
        if j == NTILE - 1:
            row = lax.broadcasted_iota(jnp.int32, (nr, UW), 0) + r0
            b = jnp.where(row == idx, _bf16_round(b + routed_update(cols)), b)
        else:
            keep = sfix_v[:, cols]
            for g in range(nr // 16):
                keep = jnp.where(fix_grp == r0 // 16 + g, s[g * 16:(g + 1) * 16], keep)
            sfix_v[:, cols] = keep
            extra = [pltpu.bitcast(keep, U32)]
        res = gated(x_v[r0:r0 + nr, cols].astype(F32), b, s)
        out_v[r0:r0 + nr, cols] = res.astype(BF16)
        if cfg['slack']['epi']:
            return 'epi', _touch([pltpu.bitcast(res, U32)] + extra)

    def out_copy(j, u):
        cols = pl.ds(0, D) if u is None else pl.ds(u * UW, UW)
        return pltpu.make_async_copy(out_v.at[pl.ds(j * T, T), cols], out_hbm.at[pl.ds(j * T, T), cols],
                                     out_sem.at[j, u or 0])

    fix_rows = pl.ds(pl.multiple_of(fix_grp * 16, 16), 16)
    fix_cp = pltpu.make_async_copy(fix_v, out_hbm.at[fix_rows], misc_sem.at[6])

    def fix_routed():
        xf = x_v[fix_rows, :].astype(F32)
        b = _bf16_round(ln_rows(xf))
        b = jnp.where(row16 + fix_grp * 16 == idx, _bf16_round(b + routed_update(slice(None))), b)
        fix_v[...] = gated(xf, b, sfix_v[...]).astype(BF16)

    steps = [(j, u) for j in range(NTILE) for u in range(NU)]
    nffn = cfg['ffn_steps']
    ffn_at = dict(zip(range(NU + 1, NU + 1 + nffn), _spread(ffn, nffn)))
    lag = NU + 1
    for n in range(len(steps) + lag + 1):
      with scope('p2_%d' % (n // NU)):
        if cfg['bar2'] and n % NU == 0 and 3 <= n // NU <= NTILE:
            out_copy(n // NU - 3, None).wait()
        if n == cfg['ffn_wait']:
            sync([], [wg_cp, wu_cp, wd_cp], 'w_ffn')()
        cur = steps[n] if n < len(steps) else None
        att = steps[n - 1] if 1 <= n <= len(steps) else None
        out = steps[n - lag] if lag <= n < len(steps) + lag else None
        epi = steps[n - lag - 1] if n > lag else None
        jobs = [{}, {}]
        for pos, job in zip(cfg['ffn_at'], ffn_at.get(n, [])):
            jobs[pos // 7].setdefault(pos % 7, []).append(job)
        epi_tasks = [P(epilogue, *epi, 2 + (n - 1) % 2, t, c) for t in (1, 0) for c in range(2)] if epi else []
        soft = [P(phi_q, cur[1], n % 2, q, t) for q in (2, 0, 3, 1) for t in range(2)] if cur else []
        terms = [P(o_terms, *att, ks) for ks in ((0, 1), (2, 3, 4), (5, 6))] if att else []
        if n == 0:
            proj(0, cur[1], cur[0], n % 2, [P(v_pack, prev[1], 1, q) for q in (2, 3, 0, 1)]
                 + [P(kv_finish, 8 + q) for q in range(4)])
            kv_update(*prev, (2, 3, 0, 1))
            held = [P(kv_finish, 12 + q) for q in range(4)] + [ffn_input] + soft
            continue
        if cur and not out:
            proj(0, cur[1], cur[0], n % 2, held)
            attend(att[1])
            run(terms)
            held = soft
            continue
        if cur:
            proj(0, cur[1], cur[0], n % 2, held + epi_tasks, jobs[0])
            held = []
            epi_tasks = []
        if att:
            attend(att[1])
        if epi and epi[1] == NU - 1 and cur:
            out_copy(epi[0], None).start()
        if out:
            if out == (NTILE - 1, 0):
                run(terms)
                terms = []
            out_proj(*out, 2 + n % 2, _merge(terms + soft, epi_tasks), jobs[1])
        else:
            run(epi_tasks)
        if epi and not cur:
            if epi[0] < NTILE - 1:
                if epi[1] == NU - 1:
                    out_copy(epi[0], None).start()
            else:
                out_copy(*epi).start()
                if epi[1] == 0:
                    for j in range(NTILE - 2 if cfg['bar2'] else 0, NTILE - 1):
                        with scope('w_o%d' % j):
                            out_copy(j, None).wait()
                    fix_routed()
                    fix_cp.start()
    pins = []
    for k, r in staged.items():
        if k.rstrip('0123') in cfg['pin'].split():
            src = r.at[(0,) * (len(r.shape) - 2) + (pl.ds(0, 8), pl.ds(0, 128))]
            pins.append(pltpu.make_async_copy(src, (pin_f if r.dtype == F32 else pin_u).at[len(pins)],
                                              pin_sem.at[len(pins)]))
            pins[-1].start()
    with scope('w_out'):
        for cp in pins:
            cp.wait()
        for u in range(NU):
            out_copy(NTILE - 1, u).wait()
        fix_cp.wait()


def make(**kw):
    cfg = dict(scopes=False, flags=None, ffn_steps=24, ffn_at=(0,1,2,3,4,5,6), kv_at=((6,(2,3,0,1)),), bar2=False, fence=0, gates='', fold_at=2, ffn_wait=5, mdl=0, dyn='sink', pin='m z kv phi vt', v_at=2, ln_pad=4, ln_k=10, lt=2, fq=2, fk=2, fv=3, vp=1, ot=2, kf=2, gin=0, gwr=1, ln=4, wo=2, ffn=0, phi=2, epi=2)
    cfg.update(kw)
    cfg['slack'] = {k: cfg[k] for k in ('ln', 'wo', 'ffn', 'phi', 'epi', 'lt', 'fq', 'fk', 'fv', 'vp', 'ot', 'kf')}

    def fn(A_x, A_wqkv, A_w_phi, A_wo, B_x, B_w_r, B_w_gate, B_w_up, B_w_down):
        del B_x
        hbm = pl.BlockSpec(memory_space=pl.ANY)
        out = pl.pallas_call(
            functools.partial(_kernel, cfg=cfg),
            in_specs=[hbm] * 8,
            out_specs=hbm,
            out_shape=jax.ShapeDtypeStruct((S, D), BF16),
            scratch_shapes=[
                pltpu.VMEM((S, D), BF16),
                pltpu.VMEM((D, 3 * D), BF16),
                pltpu.VMEM((D, DH), BF16),
                pltpu.VMEM((8, 128), BF16),
                pltpu.VMEM((D, D), BF16),
                pltpu.VMEM((D, FF), BF16),
                pltpu.VMEM((D, FF), BF16),
                pltpu.VMEM((FF, D), BF16),
                pltpu.VMEM((S, D), BF16),
                pltpu.VMEM((16, D), BF16),
                {k: pltpu.VMEM((1,) + shape, dt) for k, (shape, dt) in dict(
                    bd=((128, D), BF16), wt0=((NU, 7, 64, HD), U32), wt1=((NU, 7, 64, HD), U32),
                    wt2=((NU, 7, 64, HD), U32), wos=((NU, 7, HD // 2, 128), U32),
                    xs0=((NTILE // 2, 7, HT // 2, HD), U32), xs1=((NTILE // 2, 7, HT // 2, HD), U32),
                    xn=((S // 2, D), U32),
                    m0=((8, 128, 128), F32), m1=((8, 128, 128), F32), m2=((8, 128, 128), F32),
                    m3=((8, 128, 128), F32), phi0=((4, PR, T), U32), phi1=((4, PR, T), U32), phi2=((4, PR, T), U32), phi3=((4, PR, T), U32),
                    vt=((4, DH, T), U32), ot=((4, 4, 128, 128), F32),
                    os0=((7, HT // 2, HD), U32), os1=((7, HT // 2, HD), U32),
                    kv=((NP, PR, 128), F32), kvt=((NP, PR, 128), BF16), z=((NP, 128, 128), F32),
                    best=((NTILE * 8, 8, 128), F32), bidx=((NTILE * 8, 8, 128), jnp.int32), xb=((16, D), BF16), hb=((2, 16, 128), BF16),
                    gu=((2, 2, 2, 16, 128), F32), y=((16, D), F32), sfix=((16, D), F32), sink=((4096, 8, 128), F32), xf=((4, 2, 2, 8, D), F32)).items()},
                pltpu.VMEM((32, 8, 128), F32),
                pltpu.VMEM((32, 8, 128), U32),
                pltpu.SemaphoreType.DMA((NTILE,)),
                pltpu.SemaphoreType.DMA((3, NU)),
                pltpu.SemaphoreType.DMA((7,)),
                pltpu.SemaphoreType.DMA((NTILE, NU)),
                pltpu.SemaphoreType.DMA((32,)),
            ],
            compiler_params=pltpu.CompilerParams(vmem_limit_bytes=120 * 2**20, flags=cfg['flags']),
        )(A_x.reshape(S, D), A_wqkv, A_w_phi.reshape(D, DH), A_wo, B_w_r.reshape(8, 128),
          B_w_gate, B_w_up, B_w_down)
        return out.reshape(1, S, D)

    return fn


@jax.jit
def pallas_recurrent_scan__linear_kernel_hedgehog__moe_arch_mod__prompt_kernel(
        A_x, A_wqkv, A_w_phi, A_wo, B_x, B_w_r, B_w_gate, B_w_up, B_w_down):
    return make()(A_x, A_wqkv, A_w_phi, A_wo, B_x, B_w_r, B_w_gate, B_w_up, B_w_down)
```

```python
import contextlib
import functools

import jax
import jax.numpy as jnp
from jax import lax
import jax.experimental.pallas as pl
import jax.experimental.pallas.tpu as pltpu

F32 = jnp.float32
BF16 = jnp.bfloat16
U32 = jnp.uint32
LOG2E = 1.4426950408889634
NT = (((1,), (1,)), ((), ()))
NN = (((1,), (0,)), ((), ()))

S, D, H, DH, FF = 2048, 1024, 32, 32, 3584
NP = H // 2
PR = 2 * DH
NU = 4
UW = D // NU
FC = 256
T = 256
HT = T // 2
HD = D // 2
NTILE = S // T


def _bf16_round(v):
    return v.astype(BF16).astype(F32)


def _pack(even, odd):
    return pltpu.bitcast(pltpu.pack_elementwise([even, odd], packed_dtype=BF16), U32)


def _rows(words):
    return pltpu.bitcast(words, BF16)


def _allreduce(r, op):
    r = op(r, pltpu.roll(r, 4, 0))
    return op(r, pltpu.roll(r, 2, 0))


def _dual_exp(p):
    p3 = p.reshape(8, 8, p.shape[1])
    mx = _allreduce(jnp.max(p3, axis=0), jnp.maximum)
    mn = _allreduce(jnp.min(p3, axis=0), jnp.minimum)
    ep = jnp.exp2(p3 - mx[None])
    en = jnp.exp2(mn[None] - p3)
    rp = pl.reciprocal(_allreduce(jnp.sum(ep, axis=0), jnp.add), approx=True)
    rn = pl.reciprocal(_allreduce(jnp.sum(en, axis=0), jnp.add), approx=True)
    return ep, en, rp, rn


def _lhs_term(k, a11, a12, a21, a22):
    return (lambda: a11() + a22(), lambda: a21() + a22(), a11, a22, lambda: a11() + a12(),
            lambda: a21() - a11(), lambda: a12() - a22())[k]()


def _rhs_term(k, b11, b12, b21, b22):
    return (lambda: b11() + b22(), b11, lambda: b12() - b22(), lambda: b21() - b11(), b22,
            lambda: b11() + b12(), lambda: b21() + b22())[k]()


def _quadrant(m, r, c):
    if (r, c) == (0, 0):
        return m(0) + m(3) - m(4) + m(6)
    if (r, c) == (0, 1):
        return m(2) + m(4)
    if (r, c) == (1, 0):
        return m(1) + m(3)
    return m(0) - m(1) + m(2) + m(5)


def _better(a, b):
    take = (b[0] > a[0]) | ((b[0] == a[0]) & (b[1] < a[1]))
    return jnp.where(take, b[0], a[0]), jnp.where(take, b[1], a[1])


def _zero_after(v):
    return jnp.where(v > jnp.inf, 1.0, 0.0)


def _touch(words):
    tiles = [w[r:r + 8, c:c + 128] for w in words for r in range(0, w.shape[0], 8) for c in range(0, w.shape[1], 128)]
    return pltpu.bitcast(functools.reduce(jnp.bitwise_or, tiles), F32)


def _held(v, zero):
    if zero is None:
        return v
    z = jnp.tile(pltpu.bitcast(zero, U32), (v.shape[0] // 8, v.shape[1] // 128))
    return pltpu.bitcast(pltpu.bitcast(v, U32) | z, F32)


def _spread(tasks, nslots):
    return [tasks[s * len(tasks) // nslots:(s + 1) * len(tasks) // nslots] for s in range(nslots)]


def _merge(*lists):
    keyed = [((k + 0.5) / len(l), n, t) for n, l in enumerate(lists) for k, t in enumerate(l)]
    return [t for _, _, t in sorted(keyed, key=lambda e: e[:2])]


def _kernel(x_hbm, wqkv_hbm, wphi_hbm, wo_hbm, wr_hbm, wg_hbm, wu_hbm, wd_hbm, out_hbm,
            x_v, w_v, wphi_v, wr_v, wo_v, wg_v, wu_v, wd_v, out_v, fix_v,
            staged, pin_f, pin_u, sems, *, cfg):
    scope = lambda n: jax.named_scope(n) if (cfg['scopes'] == 1 or (cfg['scopes'] == 2 and n.startswith('w_'))) else contextlib.nullcontext()

    def x_copy(i, n, sem):
        rows = pl.ds(i * T, n * T)
        return pltpu.make_async_copy(x_hbm.at[rows], x_v.at[rows], sems.at[sem])

    def w_copy(m, u, n=1):
        cols = pl.ds(m * D + u * UW, n * UW)
        sem = 3 if m == 0 else (u + 2) % 4
        return pltpu.make_async_copy(wqkv_hbm.at[:, cols], w_v.at[:, cols], sems.at[sem])

    wr_cp = pltpu.make_async_copy(wr_hbm, wr_v, sems.at[0])
    wphi_cp = pltpu.make_async_copy(wphi_hbm, wphi_v, sems.at[2])
    x0_cp, x1_cp, x23_cp = x_copy(0, 1, 1), x_copy(1, 1, 4), x_copy(2, 2, 2)
    later = [x_copy(4, NTILE - 4, 3), w_copy(0, 0, NU), pltpu.make_async_copy(wo_hbm, wo_v, sems.at[3])]
    ffn_cps = [pltpu.make_async_copy(src, dst, sems.at[0])
               for src, dst in ((wg_hbm, wg_v), (wu_hbm, wu_v), (wd_hbm, wd_v))]

    nghost = [0]

    def ghost(v):
        k = nghost[0]
        nghost[0] += 1
        st['sink'][k] = v
        st['sink'][k] = jnp.zeros((8, 128), F32)
        return st['sink'][k]

    due = []

    def gate_of(kind, gate):
        return gate if kind in cfg['gates'].split() else None

    def run(tasks, gate=None):
        for t in tasks:
            done = t(gate)
            if done is not None and cfg['slack'][done[0]]:
                due.append([cfg['slack'][done[0]], ghost(done[1])])

    def products(slot, lhs, rhs, dims, tasks, jobs, placed=False):
        for k, group in enumerate(tasks if placed else _spread(tasks, 7)):
            words = lhs(k)
            for d in due:
                d[0] -= 1
            ready = [d[1] for d in due if d[0] <= 0]
            due[:] = [d for d in due if d[0] > 0]
            if ready:
                z = pltpu.bitcast(functools.reduce(jnp.add, ready), U32)
                last = jnp.concatenate([words[-8:, :-128], words[-8:, -128:] | z], axis=1)
                words = jnp.concatenate([words[:-8], last], axis=0)
            res = lax.dot_general(_rows(words), _rows(rhs(k)), dims, preferred_element_type=F32)
            m_v[slot][k] = res
            if cfg['mdl']:
                due.append([cfg['mdl'], ghost(_touch([pltpu.bitcast(res, U32)]))])
            if group:
                run(group, ghost(res[0:8]))
            if k == 6 and cfg['fence']:
                m_v[slot][7 + zero, 0:8, :] = res[0:8]
            for job in jobs.get(k, ()):
                job()

    def prep_bd():
        r_i = lax.broadcasted_iota(jnp.int32, (128, DH), 0)
        c_i = lax.broadcasted_iota(jnp.int32, (128, DH), 1)
        sel = ((r_i % DH) == c_i).astype(BF16)
        rep = lax.dot_general(sel, wphi_v[...], NT, preferred_element_type=F32)
        r_i = lax.broadcasted_iota(jnp.int32, (128, D), 0)
        c_i = lax.broadcasted_iota(jnp.int32, (128, D), 1)
        bd_v[...] = jnp.where((r_i // DH) == ((c_i % 128) // DH), rep, 0.0).astype(BF16)

    def fold(m, u, slot):
        for g in range(2):
            c0 = u * UW + g * 128
            t = lax.dot_general(bd_v[:, c0:c0 + 128], w_v[:, m * D + c0:m * D + c0 + 128], NT,
                                preferred_element_type=F32)
            for c in range(8):
                fold_ref(slot, g, c)[...] = t[:, c * 128:(c + 1) * 128]

    def fold_ref(slot, g, c):
        k = g * 8 + c
        return ot_v.at[k // 4, k % 4]

    def fold_terms(m, u, slot, c, q, gate):
        rows = slice(q * PR, (q + 1) * PR)
        a = [_held(fold_ref(slot, g, h * 4 + c)[rows, :], gate_of('fq', gate)) * LOG2E for g in range(2) for h in range(2)]
        outs = []
        for k in range(7):
            t = _lhs_term(k, *[(lambda v=v: v) for v in a])
            outs.append(_pack(t[:DH], t[DH:]))
            wt_v[m][u, k, q * DH:(q + 1) * DH, c * 128:(c + 1) * 128] = outs[-1]
        return 'fq' if m == 0 else 'fk', _touch(outs)

    def v_terms(u, c, ks, gate):
        c0 = 2 * D + u * UW
        blk = lambda g, h: (lambda: _held(w_v[h * HD + c * 128:h * HD + (c + 1) * 128,
                                        c0 + g * 128:c0 + (g + 1) * 128].astype(F32), gate_of('fv', gate)))
        outs = []
        for k in ks:
            t = _lhs_term(k, blk(0, 0), blk(0, 1), blk(1, 0), blk(1, 1))
            outs.append(pltpu.bitcast(t.astype(BF16).T, U32))
            wt_v[2][u, k, :, c * 128:(c + 1) * 128] = outs[-1]
        return 'fv', _touch(outs)

    def wo_terms(u, g, q, gate):
        b = [wo_v[g * UW + r * 128 + q * PR:g * UW + r * 128 + (q + 1) * PR,
                  u * UW + c * 128:u * UW + (c + 1) * 128].astype(F32) for r in range(2) for c in range(2)]
        b = [_held(v, gate_of('wo', gate)) for v in b]
        outs = []
        for k in range(7):
            t = _rhs_term(k, *[(lambda v=v: v) for v in b])
            outs.append(_pack(t[:DH], t[DH:]))
            wos_v[u, k, g * PR + q * DH:g * PR + (q + 1) * DH, :] = outs[-1]
        return 'wo', _touch(outs)

    def fold_tasks(m, u):
        return [functools.partial(fold_terms, m, u, 0, c, q) for c in range(4) for q in range(2)]

    def v_tasks_of(u):
        return [functools.partial(v_terms, u, c, ks) for ks in ((0, 1, 2), (3, 4), (5, 6)) for c in range(4)]

    def ln_rows(xf, gate=None):
        mean = jnp.sum(xf, axis=1, keepdims=True) * (1.0 / D)
        if gate is not None and cfg['gin']:
            mean = mean + gate[:, 0:1]
        cen = xf - mean
        var = jnp.sum(cen * cen, axis=1, keepdims=True) * (1.0 / D)
        den = _bf16_round(jnp.sqrt(_bf16_round(_bf16_round(var) + 1e-5)))
        return (xf - _bf16_round(mean)) * pl.reciprocal(den, approx=True)

    def ln_norm(i, c, half, e, gate):
        r0 = i * T + half * HT + c * 16
        words = pltpu.bitcast(x_v[r0:r0 + 16, :], U32)
        xf = pltpu.unpack_elementwise(words, index=e, packed_dtype=BF16, unpacked_dtype=F32)
        xn = ln_rows(_held(xf, gate_of('ln', gate)), gate)
        xf_v[c % 4, half, e] = xn
        return 'ln', _touch([pltpu.bitcast(xn, U32)])

    def ln_route(i, c, gate):
        top = None
        outs = []
        wr = wr_rows if gate is None else wr_rows + jnp.tile(gate, (1, 8))
        for half in range(2):
            r0 = i * T + half * HT + c * 16
            outs.append(_pack(xf_v[c % 4, half, 0], xf_v[c % 4, half, 1]))
            xn_v[r0 // 2:r0 // 2 + 8, :] = outs[-1]
            for e in range(2):
                r = _bf16_round(jnp.sum(xf_v[c % 4, half, e] * wr, axis=1, keepdims=True))
                r = jnp.broadcast_to(r, (8, 128))
                tok = 2 * lax.broadcasted_iota(jnp.int32, (8, 128), 0) + (r0 + e)
                if top is None:
                    top = (jnp.where(r != r, -jnp.inf, r), jnp.where(r != r, S, tok))
                else:
                    top = _better(top, (r, tok))
        best_v[i * 8 + c], bidx_v[i * 8 + c] = top
        return 'ln', _touch(outs + [pltpu.bitcast(t, U32) for t in top])

    def ln_terms(i, c, ks, gate):
        outs = []
        for k in ks:
            blk = lambda half, e, h: (lambda: _held(xf_v[c % 4, half, e, :, h * HD:(h + 1) * HD], gate_of('lt', gate)))
            t = [_rhs_term(k, blk(0, e, 0), blk(1, e, 0), blk(0, e, 1), blk(1, e, 1)) for e in range(2)]
            outs.append(_pack(*t))
            xs_v[i % 2][i // 2, k, c * 8:(c + 1) * 8, :] = outs[-1]
        return 'lt', _touch(outs)

    def ln_tasks(i):
        first = lambda c: [P(ln_norm, i, c, half, e) for half in range(2) for e in range(2)]
        second = lambda c: [P(ln_terms, i, c, (0, 1, 2)), P(ln_terms, i, c, (3, 4, 5, 6)), P(ln_route, i, c)]
        tasks = first(0)
        for c in range(1, 8):
            tasks += _merge(first(c), second(c - 1))
        return tasks + second(7)

    def proj(m, u, i, slot, tasks, jobs={}, placed=False):
        products(slot, lambda k: wt_v[m][u, k], lambda k: xs_v[i % 2][i // 2, k], NT, tasks, jobs, placed)

    def pair_block(slot, q, t):
        rows = slice((q % 2) * PR, (q % 2 + 1) * PR)
        return _quadrant(lambda k: m_v[slot][k, rows, :], q // 2, t)

    def phi_k(i, u, slot, q, t, gate):
        p = u * 4 + q
        ep, en, rp, rn = _dual_exp(_held(pair_block(slot, q, t), gate if i in cfg['hold_k'] else None))
        php = (ep * rp[None]).reshape(PR, 128)
        phn = (en * rn[None]).reshape(PR, 128)
        words = _pack(php, phn)
        phi_v[u][q, :, t * 128:(t + 1) * 128] = words
        if cfg['zmode'] and t == 0:
            return 'phi', _touch([words])
        z = jnp.concatenate([php, phn], axis=0)
        if cfg['zmode']:
            z = z + jnp.concatenate([pltpu.unpack_elementwise(phi_v[u][q, :, :128], index=e, packed_dtype=BF16,
                                                              unpacked_dtype=F32) for e in range(2)], axis=0)
        if i or (t and not cfg['zmode']):
            z = z + z_v[p]
        z_v[p] = z
        return 'phi', _touch([words, pltpu.bitcast(z, U32)])

    def v_pack(u, slot, q, gate):
        outs = []
        for t in range(2):
            vt = _held(pair_block(slot, q, t), gate_of('vp', gate))
            outs.append(_pack(vt[:DH], vt[DH:]))
            vt_v[q, :, t * 128:(t + 1) * 128] = outs[-1]
        return 'vp', _touch(outs)

    def kv_update(i, u, qs):
        for q in qs:
            upd = lax.dot_general(_rows(vt_v[q]), _rows(phi_v[u][q]), NT, preferred_element_type=F32)
            if i:
                upd = upd + kv_v[u * 4 + q]
            kv_v[u * 4 + q] = upd
            due.append([3, ghost(_touch([pltpu.bitcast(upd, U32)]))])

    def kv_finish(p, gate):
        r_i = lax.broadcasted_iota(jnp.int32, (PR, 128), 0)
        c_i = lax.broadcasted_iota(jnp.int32, (PR, 128), 1)
        zb = jnp.broadcast_to(jnp.sum(_held(z_v[p], gate_of('kf', gate)), axis=1, keepdims=True), (128, 128))
        z_v[p] = zb
        kvt_v[p] = jnp.where((r_i % 2) == ((c_i // 2) % 2), kv_v[p], 0.0).astype(BF16)
        return 'kf', _touch([pltpu.bitcast(zb, U32)])

    P = functools.partial
    nothing = lambda gate: None

    wr_cp.start()
    x0_cp.start()
    wr_cp.wait()
    wphi_cp.start()
    w_copy(1, 0).start()
    wr8 = wr_v[...].astype(F32)
    zero = jnp.where(wr8 > jnp.inf, 1, 0)[0, 0]
    wr_rows = jnp.concatenate([jnp.broadcast_to(wr8[c:c + 1], (8, 128)) for c in range(8)], axis=1)
    st = {k: r.at[zero] if (cfg['dyn'] == 'all' or k.rstrip('0123') in cfg['dyn'].split()) else r.at[0] for k, r in staged.items()}
    bd_v, wos_v, xn_v, vt_v, ot_v, kv_v, kvt_v, z_v, best_v, bidx_v, xb_v, hb_v, gu_v, y_v, sfix_v = [
        st[k] for k in 'bd wos xn vt ot kv kvt z best bidx xb hb gu y sfix'.split()]
    wt_v = [st['wt%d' % m] for m in range(3)]
    xs_v = [st['xs0'], st['xs1']]
    m_v = [st['m%d' % m] for m in range(4)]
    phi_v = [st['phi%d' % m] for m in range(4)]
    os_v = [st['os0'], st['os1']]
    xf_v = st['xf']
    w_copy(1, 1).start()
    with scope('w_x0'):
        x0_cp.wait()
    for t in ln_tasks(0):
        t(None)
    w_copy(1, 2).start()
    w_copy(1, 3).start()
    with scope('w_k0'):
        wphi_cp.wait()
        w_copy(1, 0).wait()
    prep_bd()
    fold(1, 0, 0)
    for t in fold_tasks(1, 0):
        t(None)

    def softmax_k(i, u, slot):
        return [P(phi_k, i, u, slot, q, t) for q in (2, 0, 3, 1) for t in range(2)]

    def pack_v(u, slot):
        return [P(v_pack, u, slot, q) for q in (2, 3, 0, 1)]

    def sync(starts, waits, name):
        def job():
            for cp in starts:
                cp.start()
            with scope(name):
                for cp in waits:
                    cp.wait()
        return job

    with scope('p1_0'):
        fa, va = cfg['fold_at'], cfg['v_at']
        early = cfg['x1_early']
        after = [[w_copy(2, 0)], [w_copy(2, 1)], [x1_cp], [w_copy(2, 2)]]
        for u in range(NU):
            tasks = softmax_k(0, u - 1, 2 + (u - 1) % 2) if u else []
            if u < NU - 1:
                job = [sync(after[u], [w_copy(1, u + 1)], 'w_k%d' % (u + 1)), P(fold, 1, u + 1, 0)]
                late = fold_tasks(1, u + 1)
            else:
                job = [sync(after[u], [w_copy(2, 0)], 'w_v0')]
                late = v_tasks_of(0)
            proj(1, u, 0, 2 + u % 2, _spread(tasks, fa + 1) + _spread(late, 6 - fa), {fa: job}, True)
        after = [[w_copy(2, 3)], [x23_cp],
                 later]
        need = [[w_copy(2, 1)], [w_copy(2, 2)], [w_copy(2, 3)]]
        need[0 if early else 1].append(x1_cp)
        ln = ln_tasks(1)
        c = [len(ln) * f // 16 for f in cfg['lnc']]
        ln = ([[]] * (va + 1) + _spread(ln[:c[0]], 4) + [[]] * 3 + _spread(ln[c[0]:c[1]], 4) + [[]] * 3
              + _spread(ln[c[1]:], 14 - va - 1 - 3) + [[]] * 3)
        for u in range(NU):
            tasks = softmax_k(0, NU - 1, 3) if u == 0 else pack_v(u - 1, (u - 1) % 2)
            jobs = {6: [P(kv_update, 0, u - 1, (2, 3, 0, 1))]} if u else {}
            if u + 1 < NU:
                jobs[va] = [sync(after[u], need[u], 'w_v%d' % (u + 1))]
                tasks = _spread(tasks, va + 1) + _spread(v_tasks_of(u + 1), 6 - va)
            else:
                tasks = _spread(tasks, 7)
            proj(2, u, 0, u % 2, [a + b for a, b in zip(tasks, ln[7 * u:7 * u + 7])], jobs, True)

    prev = (0, NU - 1)
    wo_tasks = [P(wo_terms, u, g, q) for u in range(NU) for g in range(4) for q in range(2)]
    for i in range(1, NTILE):
      with scope('p1_%d' % i):
        if i == 1:
            sync([], [x23_cp], 'w_x2')()
        if i == 3:
            sync(ffn_cps,
                 later, 'w_q')()
        for u in range(NU):
            k_tasks = pack_v(prev[1], 1)
            v_tasks = softmax_k(i, u, 0)
            jobs = [{}, {}]
            for pos, qs in cfg['kv_at']:
                jobs[pos // 7][pos % 7] = [P(kv_update, *prev, qs)]
            if i + 1 < NTILE:
                ln = _spread(ln_tasks(i + 1) + [nothing] * cfg['ln_pad'], NU)[u]
                nk = len(ln) * cfg['ln_k'] // 14
                k_tasks = _merge(k_tasks, ln[:nk])
                v_tasks = _merge(v_tasks, ln[nk:])
            else:
                rest = _spread(wo_tasks[4 * cfg['wo_n']:], NU)[u]
                k_tasks = _merge(k_tasks, rest)
                if u > 1:
                    k_tasks = _merge(k_tasks, [P(kv_finish, (u - 2) * 4 + q) for q in range(4)])
            if 3 <= i < 7:
                k_tasks = _merge(k_tasks, _spread(wo_tasks[(i - 3) * cfg['wo_n']:(i - 2) * cfg['wo_n']], NU)[u])
            if 3 <= i < 3 + NU:
                if u == 0:
                    jobs[0][0] = [P(fold, 0, i - 3, 0)]
                v_tasks = _merge(v_tasks, fold_tasks(0, i - 3)[2 * u:2 * u + 2])
            proj(1, u, i, 0, k_tasks, jobs[0])
            proj(2, u, i, 1, v_tasks, jobs[1])
            prev = (i, u)

    best = jnp.max(jnp.max(best_v[...], axis=0), axis=0, keepdims=True)
    bidx = jnp.min(jnp.min(jnp.where(best_v[...] == best[None], bidx_v[...], S), axis=0), axis=0, keepdims=True)
    idx_raw = bidx[0, 0]
    idx = jnp.where(idx_raw == S, 0, idx_raw)
    gate_r = _bf16_round(jax.nn.sigmoid(jnp.where(bidx == S, jnp.nan, best)))[:, 0:1]
    row16 = lax.broadcasted_iota(jnp.int32, (16, D), 0)
    grp = idx // 16
    fix_grp = jnp.where(idx >= S - T, 0, grp)

    def ffn_input(gate):
        xb_v[...] = _bf16_round(ln_rows(x_v[pl.ds(pl.multiple_of((idx // 8) * 8, 8), 8), :].astype(F32)))
        sfix_v[...] = jnp.zeros(sfix_v.shape, F32)
        return 'in', _touch([pltpu.bitcast(xb_v[...], U32)])

    def ffn_up(c, which, h):
        gu_v[c % 2, which, h] = lax.dot_general(xb_v[:, h * HD:(h + 1) * HD],
                                        (wg_v, wu_v)[which][h * HD:(h + 1) * HD, c * 128:(c + 1) * 128], NN,
                                        preferred_element_type=F32)
        if (which, h) == (1, 1):
            g = gu_v[c % 2, 0, 0] + gu_v[c % 2, 0, 1]
            hb_v[c % 2] = _bf16_round(g * jax.nn.sigmoid(g) * (gu_v[c % 2, 1, 0] + gu_v[c % 2, 1, 1]))

    def ffn_down(c, h):
        part = lax.dot_general(hb_v[c % 2], wd_v[c * 128:(c + 1) * 128, h * HD:(h + 1) * HD], NN, preferred_element_type=F32)
        if c:
            part = part + y_v[:, h * HD:(h + 1) * HD]
        y_v[:, h * HD:(h + 1) * HD] = part
        due.append([3, ghost(_touch([pltpu.bitcast(part, U32)]))])

    ffn = []
    for c in range(FF // 128):
        ffn += [P(ffn_up, c, which, h) for which in range(2) for h in range(2)]
        if c:
            ffn += [P(ffn_down, c - 1, h) for h in range(2)]
    ffn += [P(ffn_down, FF // 128 - 1, h) for h in range(2)]

    def phi_q(u, slot, q, t, hold, gate):
        p = u * 4 + q
        ep, en, rp, rn = _dual_exp(_held(pair_block(slot, q, t), gate if hold else None))
        a = jnp.sum(ep * z_v[p, :PR].reshape(8, 8, 128), axis=0)
        b = jnp.sum(en * z_v[p, PR:].reshape(8, 8, 128), axis=0)
        rd = pl.reciprocal(_allreduce(rp * a + rn * b, jnp.add) + 1e-6, approx=True)
        words = _pack((ep * (rp * rd)[None]).reshape(PR, 128), (en * (rn * rd)[None]).reshape(PR, 128))
        phi_v[u][q, :, t * 128:(t + 1) * 128] = words
        return 'phi', _touch([words])

    def attend(u, qs=(2, 3, 0, 1)):
        for q in qs:
            o = jnp.dot(kvt_v[u * 4 + q], _rows(phi_v[u][q]), preferred_element_type=F32)
            for t in range(2):
                ot_v[q // 2, t, (q % 2) * PR:(q % 2 + 1) * PR, :] = o[:, t * 128:(t + 1) * 128]

    def o_terms(j, u, ks, gate):
        blk = lambda t, g: (lambda: _held(ot_v[g, t], gate_of('ot', gate)))
        outs = []
        for k in ks:
            term = _lhs_term(k, blk(0, 0), blk(0, 1), blk(1, 0), blk(1, 1))
            outs.append(pltpu.bitcast(term.astype(BF16).T, U32))
            os_v[j % 2][k, :, u * 128:(u + 1) * 128] = outs[-1]
        return 'ot', _touch(outs)

    def out_proj(j, u, slot, tasks, jobs={}):
        products(slot, lambda k: os_v[j % 2][k], lambda k: wos_v[u, k],
                 (((1,), (0,)), ((), ())), tasks, jobs)

    def routed_update(cols):
        y = y_v[:, cols]
        mine = lax.broadcasted_iota(jnp.int32, y.shape, 0) == idx % 8
        yrow = jnp.sum(jnp.where(mine, y, 0.0), axis=0, keepdims=True)
        return _bf16_round(_bf16_round(yrow) * gate_r)

    def gated(xf, b, s):
        return xf + s * (b * pl.reciprocal(1.0 + jnp.exp2(b * (-LOG2E)), approx=True))

    def epilogue(j, u, slot, t, c, gate):
        nr = 64
        r0 = j * T + t * HT + c * nr
        cols = slice(u * UW, (u + 1) * UW)
        s = jnp.concatenate([_quadrant(lambda k: m_v[slot][k, c * nr:(c + 1) * nr, :], t, h) for h in range(2)],
                            axis=1)
        b = _held(_rows(xn_v[r0 // 2:(r0 + nr) // 2, cols]).astype(F32), gate_of('epi', gate))
        s = _held(s, gate_of('epi', gate))
        extra = []
        if j == NTILE - 1:
            row = lax.broadcasted_iota(jnp.int32, (nr, UW), 0) + r0
            b = jnp.where(row == idx, _bf16_round(b + routed_update(cols)), b)
        else:
            keep = sfix_v[:, cols]
            for g in range(nr // 16):
                keep = jnp.where(fix_grp == r0 // 16 + g, s[g * 16:(g + 1) * 16], keep)
            sfix_v[:, cols] = keep
            extra = [pltpu.bitcast(keep, U32)]
        res = gated(x_v[r0:r0 + nr, cols].astype(F32), b, s)
        out_v[r0:r0 + nr, cols] = res.astype(BF16)
        if cfg['slack']['epi']:
            return 'epi', _touch([pltpu.bitcast(res, U32)] + extra)

    def out_copy(j, u):
        cols = pl.ds(0, D) if u is None else pl.ds(u * UW, UW)
        return pltpu.make_async_copy(out_v.at[pl.ds(j * T, T), cols], out_hbm.at[pl.ds(j * T, T), cols],
                                     sems.at[4 if j < NTILE - 1 else 5])

    fix_rows = pl.ds(pl.multiple_of(fix_grp * 16, 16), 16)
    fix_cp = pltpu.make_async_copy(fix_v, out_hbm.at[fix_rows], sems.at[5])

    def fix_routed():
        xf = x_v[fix_rows, :].astype(F32)
        b = _bf16_round(ln_rows(xf))
        b = jnp.where(row16 + fix_grp * 16 == idx, _bf16_round(b + routed_update(slice(None))), b)
        fix_v[...] = gated(xf, b, sfix_v[...]).astype(BF16)

    steps = [(j, u) for j in range(NTILE) for u in range(NU)]
    nffn = cfg['ffn_steps']
    ffn_at = dict(zip(range(NU + 1, NU + 1 + nffn), _spread(ffn, nffn)))
    lag = NU + 1
    for n in range(len(steps) + lag + 1):
      with scope('p2_%d' % (n // NU)):
        if cfg['bar2'] and n % NU == 0 and 3 <= n // NU <= NTILE:
            out_copy(n // NU - 3, None).wait()
        if n == cfg['ffn_wait']:
            sync([], ffn_cps, 'w_ffn')()
        cur = steps[n] if n < len(steps) else None
        att = steps[n - 1] if 1 <= n <= len(steps) else None
        out = steps[n - lag] if lag <= n < len(steps) + lag else None
        epi = steps[n - lag - 1] if n > lag else None
        jobs = [{}, {}]
        for pos, job in zip(cfg['ffn_at'], ffn_at.get(n, [])):
            jobs[pos // 7].setdefault(pos % 7, []).append(job)
        epi_tasks = [P(epilogue, *epi, 2 + (n - 1) % 2, t, c) for t in (1, 0) for c in range(2)] if epi else []
        soft = [P(phi_q, cur[1], n % 2, q, t, n < cfg['hold_q']) for q in (2, 0, 3, 1) for t in range(2)] if cur else []
        terms = [P(o_terms, *att, ks) for ks in ((0, 1), (2, 3, 4), (5, 6))] if att else []
        if n == 0:
            proj(0, cur[1], cur[0], n % 2, [P(v_pack, prev[1], 1, q) for q in (2, 3, 0, 1)]
                 + [P(kv_finish, 8 + q) for q in range(4)])
            kv_update(*prev, (2, 3, 0, 1))
            held = [ffn_input] + _merge([P(kv_finish, 12 + q) for q in range(4)], soft)
            continue
        if cur and not out:
            proj(0, cur[1], cur[0], n % 2, _spread(held, cfg['held']) + [[]] * (7 - cfg['held']), {}, True)
            attend(att[1])
            held = _merge(terms, soft)
            continue
        if cur:
            proj(0, cur[1], cur[0], n % 2, held + epi_tasks, jobs[0])
            held = []
            epi_tasks = []
        if att:
            attend(att[1])
        if epi and epi[1] == NU - 1 and cur:
            out_copy(epi[0], None).start()
        if out:
            if out == (NTILE - 1, 0):
                run(terms)
                terms = []
            out_proj(*out, 2 + n % 2, _merge(terms + soft, epi_tasks), jobs[1])
        else:
            run(epi_tasks)
        if epi and not cur:
            if epi[0] < NTILE - 1:
                if epi[1] == NU - 1:
                    out_copy(epi[0], None).start()
            else:
                out_copy(*epi).start()
                if epi[1] == 0:
                    for j in range(NTILE - 2 if cfg['bar2'] else 0, NTILE - 1):
                        with scope('w_o%d' % j):
                            out_copy(j, None).wait()
                    fix_routed()
                    fix_cp.start()
    pins = []
    for k, r in staged.items():
        if k.rstrip('0123') in cfg['pin'].split():
            src = r.at[(0,) * (len(r.shape) - 2) + (pl.ds(0, 8), pl.ds(0, 128))]
            pins.append(pltpu.make_async_copy(src, (pin_f if r.dtype == F32 else pin_u).at[len(pins)],
                                              sems.at[5]))
            pins[-1].start()
    with scope('w_out'):
        for cp in pins:
            cp.wait()
        for u in range(NU):
            out_copy(NTILE - 1, u).wait()
        fix_cp.wait()


def make(**kw):
    cfg = dict(scopes=False, flags=None, ffn_steps=24, ffn_at=(0,1,2,3,4,5,6), kv_at=((6,(2,3,0,1)),), bar2=False, lnc=(4, 8), x1_early=1, hold_k=(7,), hold_q=4, held=6, wo_n=2, zmode=1, fence=0, gates='', fold_at=2, ffn_wait=5, mdl=0, dyn='sink', pin='m z kv phi vt', v_at=2, ln_pad=4, ln_k=8, lt=2, fq=2, fk=2, fv=3, vp=1, ot=2, kf=2, gin=0, gwr=1, ln=4, wo=2, ffn=2, phi=2, epi=2)
    cfg['in'] = 5
    cfg.update(kw)
    cfg['slack'] = {k: cfg[k] for k in ('ln', 'wo', 'ffn', 'phi', 'epi', 'in', 'lt', 'fq', 'fk', 'fv', 'vp', 'ot', 'kf')}

    def fn(A_x, A_wqkv, A_w_phi, A_wo, B_x, B_w_r, B_w_gate, B_w_up, B_w_down):
        del B_x
        hbm = pl.BlockSpec(memory_space=pl.ANY)
        out = pl.pallas_call(
            functools.partial(_kernel, cfg=cfg),
            in_specs=[hbm] * 8,
            out_specs=hbm,
            out_shape=jax.ShapeDtypeStruct((S, D), BF16),
            scratch_shapes=[
                pltpu.VMEM((S, D), BF16),
                pltpu.VMEM((D, 3 * D), BF16),
                pltpu.VMEM((D, DH), BF16),
                pltpu.VMEM((8, 128), BF16),
                pltpu.VMEM((D, D), BF16),
                pltpu.VMEM((D, FF), BF16),
                pltpu.VMEM((D, FF), BF16),
                pltpu.VMEM((FF, D), BF16),
                pltpu.VMEM((S, D), BF16),
                pltpu.VMEM((16, D), BF16),
                {k: pltpu.VMEM((1,) + shape, dt) for k, (shape, dt) in dict(
                    bd=((128, D), BF16), wt0=((NU, 7, 64, HD), U32), wt1=((NU, 7, 64, HD), U32),
                    wt2=((NU, 7, 64, HD), U32), wos=((NU, 7, HD // 2, 128), U32),
                    xs0=((NTILE // 2, 7, HT // 2, HD), U32), xs1=((NTILE // 2, 7, HT // 2, HD), U32),
                    xn=((S // 2, D), U32),
                    m0=((8, 128, 128), F32), m1=((8, 128, 128), F32), m2=((8, 128, 128), F32),
                    m3=((8, 128, 128), F32), phi0=((4, PR, T), U32), phi1=((4, PR, T), U32), phi2=((4, PR, T), U32), phi3=((4, PR, T), U32),
                    vt=((4, DH, T), U32), ot=((4, 4, 128, 128), F32),
                    os0=((7, HT // 2, HD), U32), os1=((7, HT // 2, HD), U32),
                    kv=((NP, PR, 128), F32), kvt=((NP, PR, 128), BF16), z=((NP, 128, 128), F32),
                    best=((NTILE * 8, 8, 128), F32), bidx=((NTILE * 8, 8, 128), jnp.int32), xb=((8, D), F32), hb=((2, 8, 128), F32),
                    gu=((2, 2, 2, 8, 128), F32), y=((8, D), F32), sfix=((16, D), F32), sink=((4096, 8, 128), F32), xf=((4, 2, 2, 8, D), F32)).items()},
                pltpu.VMEM((32, 8, 128), F32),
                pltpu.VMEM((32, 8, 128), U32),
                pltpu.SemaphoreType.DMA((6,)),
            ],
            compiler_params=pltpu.CompilerParams(vmem_limit_bytes=120 * 2**20, flags=cfg['flags']),
        )(A_x.reshape(S, D), A_wqkv, A_w_phi.reshape(D, DH), A_wo, B_w_r.reshape(8, 128),
          B_w_gate, B_w_up, B_w_down)
        return out.reshape(1, S, D)

    return fn


@jax.jit
def pallas_recurrent_scan__linear_kernel_hedgehog__moe_arch_mod__prompt_kernel(
        A_x, A_wqkv, A_w_phi, A_wo, B_x, B_w_r, B_w_gate, B_w_up, B_w_down):
    return make()(A_x, A_wqkv, A_w_phi, A_wo, B_x, B_w_r, B_w_gate, B_w_up, B_w_down)
```

```python
import functools

import jax
import jax.numpy as jnp
from jax import lax
import jax.experimental.pallas as pl
import jax.experimental.pallas.tpu as pltpu

F32 = jnp.float32
BF16 = jnp.bfloat16
U32 = jnp.uint32
LOG2E = 1.4426950408889634
NN = (((1,), (0,)), ((), ()))
NT = (((1,), (1,)), ((), ()))

S, D, H, FF = 2048, 1024, 32, 3584
DH = D // H
HD = D // 2
PR = 2 * DH
NU = 4
UW = D // NU
T = 256
HT = T // 2
NTILE = S // T
NPROD = 7
NORDER = 1024
PAIRS = (2, 3, 0, 1)
P = functools.partial
CFG = dict(ln=4, l1=4, lt=3, fq=2, fk=3, fv=4, wo=3, phi=3, epi=2, vp=2, ot=2, kf=3, ln_k=10, ln_pad=4, gap=3,
           lnc=(4, 8), pin='m z kv phi vt wt wos os', wo_n=0, late=0, kv7=6, plain=[(7, u) for u in range(4)], hq=4, hk=(3,4,5,6,7), wh=6, e0=0, xf=0, fqk=0)


def _dot(a, b, dims=NN):
    return lax.dot_general(a, b, dims, preferred_element_type=F32)


def _bf16_round(v):
    return v.astype(BF16).astype(F32)


def _recip(v):
    return pltpu.reciprocal(v, approx=True)


def _transposed_words(v):
    return pltpu.bitcast(v.astype(BF16).T, U32)


def _pair_reduce(r, op):
    r = op(r, pltpu.roll(r, 4, 0))
    return op(r, pltpu.roll(r, 2, 0))


def _dual_exp(p):
    p3 = p.reshape(8, 8, 128)
    top = _pair_reduce(jnp.max(p3, axis=0), jnp.maximum)
    low = _pair_reduce(jnp.min(p3, axis=0), jnp.minimum)
    e_pos = jnp.exp2(p3 - top[None])
    e_neg = jnp.exp2(low[None] - p3)
    r_pos = _recip(_pair_reduce(jnp.sum(e_pos, axis=0), jnp.add))
    r_neg = _recip(_pair_reduce(jnp.sum(e_neg, axis=0), jnp.add))
    return e_pos, e_neg, r_pos, r_neg


def _features(e_pos, e_neg, r_pos, r_neg):
    return jnp.concatenate([(e_pos * r_pos[None]).reshape(PR, 128), (e_neg * r_neg[None]).reshape(PR, 128)], axis=0)


def _lhs_term(k, a):
    return (lambda: a(0, 0) + a(1, 1), lambda: a(1, 0) + a(1, 1), lambda: a(0, 0), lambda: a(1, 1),
            lambda: a(0, 0) + a(0, 1), lambda: a(1, 0) - a(0, 0), lambda: a(0, 1) - a(1, 1))[k]()


def _rhs_term(k, b):
    return (lambda: b(0, 0) + b(1, 1), lambda: b(0, 0), lambda: b(0, 1) - b(1, 1), lambda: b(1, 0) - b(0, 0),
            lambda: b(1, 1), lambda: b(0, 0) + b(0, 1), lambda: b(1, 0) + b(1, 1))[k]()


def _quadrant(m, i, j):
    if (i, j) == (0, 0):
        return m(0) + m(3) - m(4) + m(6)
    if (i, j) == (0, 1):
        return m(2) + m(4)
    if (i, j) == (1, 0):
        return m(1) + m(3)
    return m(0) - m(1) + m(2) + m(5)


def _layernorm(xf):
    mean = jnp.sum(xf, axis=1, keepdims=True) * (1.0 / D)
    cen = xf - mean
    var = jnp.sum(cen * cen, axis=1, keepdims=True) * (1.0 / D)
    den = _bf16_round(jnp.sqrt(_bf16_round(_bf16_round(var) + 1e-5)))
    return (xf - _bf16_round(mean)) * _recip(den)


def _gated(xf, b, s):
    return xf + s * (b * _recip(1.0 + jnp.exp2(b * (-LOG2E))))


def _touch(*arrays):
    words = [a if a.dtype == U32 else pltpu.bitcast(a, U32) for a in arrays]
    tiles = [w[r:r + 8, c:c + 128] for w in words for r in range(0, w.shape[0], 8) for c in range(0, w.shape[1], 128)]
    return functools.reduce(jnp.bitwise_or, tiles)


def _spread(tasks, lo=0, hi=NPROD, slots=NPROD):
    n = hi - lo
    return [[]] * lo + [tasks[s * len(tasks) // n:(s + 1) * len(tasks) // n] for s in range(n)] + [[]] * (slots - hi)


def _join(*plans):
    return [sum(groups, []) for groups in zip(*plans)]


def _merge(*lists):
    keyed = [((k + 0.5) / len(l), n, t) for n, l in enumerate(lists) for k, t in enumerate(l)]
    return [t for _, _, t in sorted(keyed, key=lambda e: e[:2])]


def _kernel(x_hbm, wqkv_hbm, wphi_hbm, wo_hbm, wr_hbm, wg_hbm, wu_hbm, wd_hbm, out_hbm,
            x_v, w_v, wphi_v, wr_v, wo_v, wg_v, wu_v, wd_v, out_v, fix_v, work, sems):
    bd_v, fold_v, wt_v, xn_v, score_v, best_v, bidx_v = [work[k] for k in 'bd fold wt xn score best bidx'.split()]
    vt_v, kv_v, kvt_v, z_v, ot_v = [work[k] for k in 'vt kv kvt z ot'.split()]
    xsel_v, gu_v, h_v, y_v, sfix_v = [work[k] for k in 'xsel gu h y sfix'.split()]
    xs_v, wos_v = work['xs'], work['wos']
    phi_v = [work['phi%d' % k] for k in range(NU)]
    m_v = [work['m%d' % k] for k in range(4)]
    os_v = [work['os%d' % k] for k in range(2)]

    def copy(src, dst, sem):
        return pltpu.make_async_copy(src, dst, sems.at[sem])

    def x_copy(r0, n, sem):
        return copy(x_hbm.at[pl.ds(r0, n)], x_v.at[pl.ds(r0, n)], sem)

    def w_copy(c0, n, sem):
        return copy(wqkv_hbm.at[:, pl.ds(c0, n)], w_v.at[:, pl.ds(c0, n)], sem)

    def k_copies(u):
        rows = pl.ds(UW, D - UW) if u else pl.ds(0, UW)
        phi = [copy(wphi_hbm.at[rows], wphi_v.at[rows], (u + 2) % 4)] if u < 2 else []
        return [w_copy(D + u * UW, UW, (u + 2) % 4)] + phi

    def v_copy(u):
        return w_copy(2 * D + u * UW, UW, (u + 2) % 4)

    def out_copy(j, u=None, t=None):
        rows = pl.ds(j * T, T) if t is None else pl.ds(j * T + t * HT, HT)
        cols = pl.ds(0, D) if u is None else pl.ds(u * UW, UW)
        return copy(out_v.at[rows, cols], out_hbm.at[rows, cols], 4 if j < NTILE - 1 else 5)

    def sync(starts, waits):
        for cp in starts:
            cp.start()
        for cp in waits:
            cp.wait()

    wr_cp = copy(wr_hbm, wr_v, 0)
    x0_cps = [x_copy(0, HT, 1), x_copy(HT, HT, 4)]
    x1_cp, x23_cp = x_copy(T, T, 4), x_copy(2 * T, 2 * T, 2)
    later_cps = [x_copy(4 * T, S - 4 * T, 3), w_copy(0, D, 3), copy(wo_hbm, wo_v, 3)]
    ffn_cps = [copy(wg_hbm, wg_v, 0), copy(wu_hbm, wu_v, 0), copy(wd_hbm, wd_v, 0)]

    sync([wr_cp] + x0_cps, [wr_cp])
    wr8 = wr_v[...].astype(F32)
    wr_rows = jnp.concatenate([jnp.broadcast_to(wr8[c:c + 1], (8, 128)) for c in range(8)], axis=1)

    order_v = work['order'].at[jnp.where(wr8 > jnp.inf, 1, 0)[0, 0]]
    count = [0]
    due = []

    def after(v):
        k = count[0] % NORDER
        count[0] += 1
        order_v[k] = v
        order_v[k] = jnp.zeros((8, 128), U32)
        return order_v[k]

    def finish_within(products, v):
        due.append([products, after(v)])

    def run(tasks):
        for task in tasks:
            task(None)

    def products(slot, lhs, rhs, dims, plan, jobs):
        for k in range(NPROD):
            for d in due:
                d[0] -= 1
            ready = [d[1] for d in due if d[0] <= 0]
            due[:] = [d for d in due if d[0] > 0]
            words = lhs(k)
            if ready:
                zero = functools.reduce(jnp.bitwise_or, ready)
                last = jnp.concatenate([words[-8:, :-128], words[-8:, -128:] | zero], axis=1)
                words = jnp.concatenate([words[:-8], last], axis=0)
            res = _dot(pltpu.bitcast(words, BF16), rhs(k), dims)
            m_v[slot][k] = res
            if plan[k]:
                begun = pltpu.bitcast(after(pltpu.bitcast(res[0:8], U32)), F32)
                for task in plan[k]:
                    done = task(begun)
                    if done is not None:
                        finish_within(*done)
            for job in jobs.get(k, ()):
                job()

    def block(slot, i, j, rows):
        return _quadrant(lambda k: m_v[slot][k, rows, :], i, j)

    def pair_block(slot, q, t):
        return block(slot, q // 2, t, slice((q % 2) * PR, (q % 2 + 1) * PR))

    def held(v, begun):
        return v if begun is None else v + jnp.tile(begun, (v.shape[0] // 8, v.shape[1] // 128))

    idle = [lambda begun: None]

    def prep_phi(lo, hi):
        r_i = lax.broadcasted_iota(jnp.int32, (128, DH), 0)
        c_i = lax.broadcasted_iota(jnp.int32, (128, DH), 1)
        rep = _dot(((r_i % PR) // 2 == c_i).astype(BF16), wphi_v[lo:hi], NT)
        r_i = lax.broadcasted_iota(jnp.int32, rep.shape, 0)
        c_i = lax.broadcasted_iota(jnp.int32, rep.shape, 1)
        bd_v[:, lo:hi] = jnp.where((r_i // PR) * 2 + r_i % 2 == (c_i % 128) // DH, rep, 0.0).astype(BF16)

    def fold(m, u):
        for g in range(2):
            c0 = u * UW + g * 128
            t = _dot(bd_v[:, c0:c0 + 128], w_v[:, m * D + c0:m * D + c0 + 128], NT) * LOG2E
            fold_v[g] = t

    def proj_terms(m, u, c, ks, begun):
        cols = lambda h: slice(h * HD + c * 128, h * HD + (c + 1) * 128)
        if m < 2 and CFG['xf']:
            outs = [_transposed_words(_lhs_term(k, lambda g, h: fold_v[g, :, cols(h)].T)) for k in ks]
        elif m < 2:
            outs = [pltpu.bitcast(_lhs_term(k, lambda g, h: fold_v[g, :, cols(h)]).astype(BF16), U32) for k in ks]
        else:
            c0 = 2 * D + u * UW
            blk = lambda g, h: w_v[cols(h), c0 + g * 128:c0 + (g + 1) * 128].astype(F32)
            outs = [_transposed_words(_lhs_term(k, blk)) for k in ks]
        for k, words in zip(ks, outs):
            wt_v[m, u, k, :, c * 128:(c + 1) * 128] = words
        return CFG['fv' if m == 2 else 'fk' if m else 'fq'], _touch(*outs)

    def weight_tasks(m, u):
        return [P(proj_terms, m, u, c, ks) for ks in ((0, 1, 2), (3, 4), (5, 6)) for c in range(4)]

    def wo_terms(u, g, ks, begun):
        blk = lambda i, j: wo_v[g * UW + i * 128:g * UW + (i + 1) * 128,
                                u * UW + j * 128:u * UW + (j + 1) * 128].astype(F32)
        outs = [pltpu.bitcast(_rhs_term(k, blk).astype(BF16), U32) for k in ks]
        for k, words in zip(ks, outs):
            wos_v[u, k, g * 64:(g + 1) * 64, :] = words
        return CFG['wo'], _touch(*outs)

    def ln_norm(g, begun):
        xn = _layernorm(x_v[g * 8:(g + 1) * 8, :].astype(F32))
        xn_v[g * 8:(g + 1) * 8, :] = xn.astype(BF16)
        r = jnp.broadcast_to(_bf16_round(jnp.sum(xn * held(wr_rows, begun), axis=1, keepdims=True)), (8, 128))
        score_v[g] = r
        return CFG['ln' if g >= 64 else 'l1'], _touch(xn, r)

    def ln_best(i, begun):
        best = jnp.full((8, 128), -jnp.inf, F32)
        first = jnp.full((8, 128), S, jnp.int32)
        for g in range(i * T // 8, (i + 1) * T // 8):
            r = score_v[g]
            tok = lax.broadcasted_iota(jnp.int32, (8, 128), 0) + g * 8
            take = (r > best) | ((r == best) & (tok < first))
            best, first = jnp.where(take, r, best), jnp.where(take, tok, first)
        best_v[i], bidx_v[i] = best, first
        return CFG['ln'], _touch(best, first)

    x_ops = {}

    def ln_terms(i, c, begun):
        blk = lambda h, t: xn_v[i * T + t * HT + c * 16:i * T + t * HT + (c + 1) * 16, h * HD:(h + 1) * HD].astype(F32)
        outs = {k: _rhs_term(k, blk) for k in (0, 2, 3, 5, 6)}
        for k, term in outs.items():
            xs_v[i, k, c * 16:(c + 1) * 16, :] = term.astype(BF16)
        return CFG['lt'], _touch(*outs.values())

    def x_operand(i, k):
        if (i, k) not in x_ops:
            if k in (1, 4):
                t = k // 4
                x_ops[i, k] = xn_v[i * T + t * HT:i * T + (t + 1) * HT, t * HD:(t + 1) * HD]
            else:
                x_ops[i, k] = xs_v[i, k]
        return x_ops[i, k]

    def ln_tasks(i):
        norm = lambda c: [P(ln_norm, (i * T + t * HT + c * 16) // 8 + e) for t in range(2) for e in range(2)]
        tasks = norm(0)
        for c in range(1, HT // 16):
            tasks += norm(c)[:3] + [P(ln_terms, i, c - 1)] + norm(c)[3:]
        return tasks + idle * CFG['gap'] + [P(ln_terms, i, HT // 16 - 1), P(ln_best, i)]

    def proj(m, u, i, slot, plan, jobs=None):
        products(slot, lambda k: wt_v[m, u, k], lambda k: x_operand(i, k), NT, plan, jobs or {})

    def keep_features(u, q, t, f, turn=True):
        words = _transposed_words(f) if turn else pltpu.bitcast(f.astype(BF16), U32)
        phi_v[u][q, t * (HT // 2):(t + 1) * (HT // 2), :] = words
        return words

    def phi_k(i, u, slot, q, t, begun):
        f = _features(*_dual_exp(held(pair_block(slot, q, t), begun if i in CFG['hk'] else None)))
        words = keep_features(u, q, t, f, (i, u) not in CFG['plain'])
        z = f + z_v[u * 4 + q] if i or t else f
        z_v[u * 4 + q] = z
        return CFG['phi'], _touch(z, words)

    def v_round(u, slot, q, begun):
        v = jnp.concatenate([pair_block(slot, q, t) for t in range(2)], axis=1)
        vt_v[q] = v.astype(BF16)
        return CFG['vp'], _touch(v)

    def features(u, q):
        return pltpu.bitcast(phi_v[u][q], BF16)

    def kv_update(i, u):
        for q in PAIRS:
            if (i, u) in CFG['plain']:
                words = jnp.concatenate([phi_v[u][q, :PR], phi_v[u][q, PR:]], axis=1)
                acc = _dot(vt_v[q], pltpu.bitcast(words, BF16), NT)
            else:
                acc = _dot(vt_v[q], features(u, q))
            if i:
                acc = acc + kv_v[u * 4 + q]
            kv_v[u * 4 + q] = acc
            finish_within(3, _touch(acc))

    def kv_finish(p, begun):
        r_i = lax.broadcasted_iota(jnp.int32, (PR, 128), 0)
        c_i = lax.broadcasted_iota(jnp.int32, (PR, 128), 1)
        z = jnp.broadcast_to(jnp.sum(z_v[p], axis=1, keepdims=True), (128, 128))
        z_v[p] = z
        kvt_v[p] = jnp.where(r_i // DH == c_i % 2, kv_v[p], 0.0).astype(BF16)
        return CFG['kf'], _touch(z)

    def key_tasks(i, u, slot):
        return [P(phi_k, i, u, slot, q, t) for q in PAIRS for t in range(2)]

    def value_tasks(u, slot):
        return [P(v_round, u, slot, q) for q in PAIRS]

    sync(k_copies(0), x0_cps[:1])
    sync(k_copies(1), x0_cps[1:])
    run(ln_tasks(0))
    sync(k_copies(2), k_copies(0))
    prep_phi(0, UW)
    fold(1, 0)
    run(weight_tasks(1, 0))
    starts = [k_copies(3), [v_copy(0)], [v_copy(1), x1_cp], [v_copy(2)]]
    for u in range(NU):
        a = 2 if u else 3
        if u + 1 < NU:
            job = [P(sync, starts[u], k_copies(u + 1))] + ([] if u else [P(prep_phi, UW, D)]) + [P(fold, 1, u + 1)]
            late = weight_tasks(1, u + 1)
        else:
            job = [P(sync, starts[u], [v_copy(0)])]
            late = weight_tasks(2, 0)
        early = key_tasks(0, u - 1, 2 + (u - 1) % 2) if u else []
        proj(1, u, 0, 2 + u % 2, _join(_spread(early, 0, a + 1), _spread(late, a + 1)), {a: job})
    starts = [[v_copy(3)], [x23_cp], later_cps]
    waits = [[v_copy(1), x1_cp], [v_copy(2)], [v_copy(3)]]
    ln = ln_tasks(1)
    c0, c1 = [len(ln) * f // 16 for f in CFG['lnc']]
    ln = _join(_spread(ln[:c0], 3, 7, 28), _spread(ln[c0:c1], 10, 14, 28), _spread(ln[c1:], 17, 25, 28))
    for u in range(NU):
        early = value_tasks(u - 1, (u - 1) % 2) if u else key_tasks(0, NU - 1, 3)
        jobs = {NPROD - 1: [P(kv_update, 0, u - 1)]} if u else {}
        plan = _spread(early)
        if u + 1 < NU:
            jobs[2] = [P(sync, starts[u], waits[u])]
            plan = _join(_spread(early, 0, 3), _spread(weight_tasks(2, u + 1), 3))
        proj(2, u, 0, u % 2, _join(plan, ln[NPROD * u:NPROD * (u + 1)]), jobs)

    wo_tasks = [P(wo_terms, u, g, ks) for u in range(NU) for g in range(NU) for ks in ((0, 1, 2), (3, 4, 5, 6))]
    prev = (0, NU - 1)
    for i in range(1, NTILE):
        if i == 1:
            sync([], [x23_cp])
        if i == 3:
            sync(ffn_cps, later_cps)
        side = ln_tasks(i + 1) + idle * CFG['ln_pad'] if i + 1 < NTILE else wo_tasks[4 * CFG['wo_n']:]
        for u in range(NU):
            mine = side[u * len(side) // NU:(u + 1) * len(side) // NU]
            cut = len(mine) * CFG['ln_k'] // 14 if i + 1 < NTILE else len(mine)
            k_tasks = _merge(value_tasks(prev[1], 1), mine[:cut])
            v_tasks = _merge(key_tasks(i, u, 0), mine[cut:])
            k_jobs = {NPROD - 1: [P(kv_update, *prev)]}
            if 3 <= i < 3 + NU:
                if u == 0:
                    k_jobs[0] = [P(fold, 0, i - 3)]
                k_tasks = _merge(k_tasks, weight_tasks(0, i - 3)[3 * u:3 * u + 3]) if CFG['fqk'] and u else k_tasks
                v_tasks = v_tasks if CFG['fqk'] and u else _merge(v_tasks, weight_tasks(0, i - 3)[3 * u:3 * u + 3])
                n = CFG['wo_n']
                k_tasks = _merge(k_tasks, wo_tasks[(i - 3) * n + u * n // NU:(i - 3) * n + (u + 1) * n // NU])
            if i == NTILE - 1 and u > 1:
                k_tasks = _merge(k_tasks, [P(kv_finish, (u - 2) * 4 + q) for q in range(4)])
            proj(1, u, i, 0, _spread(k_tasks), k_jobs)
            proj(2, u, i, 1, _spread(v_tasks))
            prev = (i, u)

    best = jnp.max(jnp.max(best_v[...], axis=0), axis=0, keepdims=True)
    first = jnp.min(jnp.min(jnp.where(best_v[...] == best[None], bidx_v[...], S), axis=0), axis=0, keepdims=True)
    idx = jnp.where(first[0, 0] == S, 0, first[0, 0])
    route_gate = _bf16_round(jax.nn.sigmoid(jnp.where(first == S, jnp.nan, best)))[:, 0:1]
    fix_grp = jnp.where(idx >= S - T, 0, idx // 16)
    fix_rows = pl.ds(pl.multiple_of(fix_grp * 16, 16), 16)
    fix_cp = copy(fix_v, out_hbm.at[fix_rows], 5)

    def ffn_input(begun):
        xsel = _bf16_round(_layernorm(x_v[pl.ds(pl.multiple_of((idx // 8) * 8, 8), 8), :].astype(F32)))
        xsel_v[...] = xsel
        sfix_v[...] = jnp.zeros(sfix_v.shape, F32)
        return 5, _touch(xsel)

    def ffn_up(c, which, h):
        half = slice(h * HD, (h + 1) * HD)
        gu_v[c % 2, which, h] = _dot(xsel_v[:, half], (wg_v, wu_v)[which][half, c * 128:(c + 1) * 128])
        if which and h:
            g = gu_v[c % 2, 0, 0] + gu_v[c % 2, 0, 1]
            h_v[c % 2] = _bf16_round(g * jax.nn.sigmoid(g) * (gu_v[c % 2, 1, 0] + gu_v[c % 2, 1, 1]))

    def ffn_down(c, h):
        half = slice(h * HD, (h + 1) * HD)
        y = _dot(h_v[c % 2], wd_v[c * 128:(c + 1) * 128, half])
        if c:
            y = y + y_v[:, half]
        y_v[:, half] = y
        finish_within(3, _touch(y))

    ffn = []
    for c in range(FF // 128):
        ffn += [P(ffn_up, c, which, h) for which in range(2) for h in range(2)]
        ffn += [P(ffn_down, c - 1, h) for h in range(2)] if c else []
    ffn += [P(ffn_down, FF // 128 - 1, h) for h in range(2)]

    def routed_update(cols):
        y = y_v[:, cols]
        mine = lax.broadcasted_iota(jnp.int32, y.shape, 0) == idx % 8
        return _bf16_round(_bf16_round(jnp.sum(jnp.where(mine, y, 0.0), axis=0, keepdims=True)) * route_gate)

    def fix_routed():
        b = xn_v[fix_rows, :].astype(F32)
        row = lax.broadcasted_iota(jnp.int32, b.shape, 0) + fix_grp * 16
        b = jnp.where(row == idx, _bf16_round(b + routed_update(slice(None))), b)
        fix_v[...] = _gated(x_v[fix_rows, :].astype(F32), b, sfix_v[...]).astype(BF16)

    def phi_q(u, slot, q, t, hold, begun):
        e_pos, e_neg, r_pos, r_neg = _dual_exp(held(pair_block(slot, q, t), begun if hold else None))
        a = jnp.sum(e_pos * z_v[u * 4 + q, :PR].reshape(8, 8, 128), axis=0)
        b = jnp.sum(e_neg * z_v[u * 4 + q, PR:].reshape(8, 8, 128), axis=0)
        r_den = _recip(_pair_reduce(r_pos * a + r_neg * b, jnp.add) + 1e-6)
        f = _features(e_pos, e_neg, r_pos * r_den, r_neg * r_den)
        return CFG['phi'], _touch(keep_features(u, q, t, f))

    def attend(u):
        for q in PAIRS:
            o = _dot(kvt_v[u * 4 + q], features(u, q), NT)
            for t in range(2):
                ot_v[q // 2, t, (q % 2) * PR:(q % 2 + 1) * PR, :] = o[:, t * 128:(t + 1) * 128]

    def o_terms(j, u, ks, begun):
        outs = [_transposed_words(_lhs_term(k, lambda t, g: ot_v[g, t])) for k in ks]
        for k, words in zip(ks, outs):
            os_v[j % 2][k, :, u * 128:(u + 1) * 128] = words
        return CFG['ot'], _touch(*outs)

    def out_proj(j, u, slot, plan):
        products(slot, lambda k: os_v[j % 2][k], lambda k: pltpu.bitcast(wos_v[u, k], BF16), NN, plan, {})

    def epilogue(j, u, slot, t, c, begun):
        r0 = j * T + t * HT + c * 64
        cols = slice(u * UW, (u + 1) * UW)
        s = jnp.concatenate([block(slot, t, h, slice(c * 64, (c + 1) * 64)) for h in range(2)], axis=1)
        b = xn_v[r0:r0 + 64, cols].astype(F32)
        kept = []
        if j == NTILE - 1:
            row = lax.broadcasted_iota(jnp.int32, b.shape, 0) + r0
            b = jnp.where(row == idx, _bf16_round(b + routed_update(cols)), b)
        else:
            keep = sfix_v[:, cols]
            for g in range(4):
                keep = jnp.where(fix_grp == r0 // 16 + g, s[g * 16:(g + 1) * 16], keep)
            sfix_v[:, cols] = keep
            kept = [keep]
        res = _gated(x_v[r0:r0 + 64, cols].astype(F32), b, s)
        out_v[r0:r0 + 64, cols] = res.astype(BF16)
        return CFG['epi'], _touch(res, *kept)

    steps = [(j, u) for j in range(NTILE) for u in range(NU)]
    lag = NU + 1
    waiting = []
    for n in range(len(steps) + lag + 1):
        cur = steps[n] if n < len(steps) else None
        att = steps[n - 1] if 1 <= n <= len(steps) else None
        out = steps[n - lag] if lag <= n < len(steps) + lag else None
        epi = steps[n - lag - 1] if n > lag else None
        ends = [P(epilogue, *epi, 2 + (n - 1) % 2, t, c) for t in (1, 0) for c in range(2)] if epi else []
        soft = [P(phi_q, cur[1], n % 2, q, t, n < CFG['hq']) for q in PAIRS for t in range(2)] if cur else []
        terms = [P(o_terms, *att, ks) for ks in ((0, 1), (2, 3, 4), (5, 6))] if att else []
        if n == lag:
            sync([], ffn_cps)
        if n == 0:
            plan = _join(_spread(value_tasks(prev[1], 1), 0, 3), _spread([P(kv_finish, 8 + q) for q in range(4)], 3))
            proj(0, cur[1], cur[0], 0, plan, {CFG['kv7']: [P(kv_update, *prev)]})
            waiting = [ffn_input] + _merge([P(kv_finish, 12 + q) for q in range(4)], soft)
        elif not out and cur:
            proj(0, cur[1], cur[0], n % 2, _spread(waiting, 0, CFG['wh']))
            attend(att[1])
            waiting = _merge(terms, soft)
        elif cur:
            jobs = {k: [job] for k, job in enumerate(ffn[(n - lag) * NPROD:(n - lag + 1) * NPROD])}
            proj(0, cur[1], cur[0], n % 2, _join(_spread(waiting, 0, 5), _spread(ends, CFG['e0'])), jobs)
            waiting = terms if CFG['late'] and cur != steps[-1] else []
            attend(att[1])
            if epi and epi[1] == NU - 1:
                out_copy(epi[0]).start()
            out_proj(*out, 2 + n % 2, _spread(soft if waiting else terms + soft))
        elif out:
            if att:
                attend(att[1])
            out_proj(*out, 2 + n % 2, _spread(_merge(terms, ends)))
            if epi == (NTILE - 2, NU - 1):
                out_copy(epi[0]).start()
            if epi[0] == NTILE - 1:
                out_copy(*epi).start()
            if epi == (NTILE - 1, 0):
                sync([], [out_copy(j) for j in range(NTILE - 1)])
                fix_routed()
                fix_cp.start()
        else:
            for k, t in enumerate((1, 0)):
                run(ends[2 * k:2 * k + 2])
                out_copy(*epi, t).start()

    pins = [r for k, r in work.items() if k.rstrip('0123') in CFG['pin'].split()]
    pins = [copy(r.at[(0,) * (len(r.shape) - 2) + (pl.ds(0, 8), pl.ds(0, 128))], work[r.dtype.name].at[k], 5)
            for k, r in enumerate(pins)]
    sync(pins, pins + [fix_cp] + [out_copy(NTILE - 1, u) for u in range(NU - 1)]
         + [out_copy(NTILE - 1, NU - 1, t) for t in range(2)])


def _call(A_x, A_wqkv, A_w_phi, A_wo, B_x, B_w_r, B_w_gate, B_w_up, B_w_down):
    del B_x
    work = dict(
        order=((1, NORDER, 8, 128), U32), float32=((16, 8, 128), F32), uint32=((16, 8, 128), U32),
        bfloat16=((16, 8, 128), BF16),
        bd=((128, D), BF16), fold=((2, 128, D), F32), wt=((3, NU, NPROD, 64, HD), U32),
        xn=((S, D), BF16), score=((S // 8, 8, 128), F32),
        best=((NTILE, 8, 128), F32), bidx=((NTILE, 8, 128), jnp.int32),
        kv=((H // 2, PR, 128), F32), kvt=((H // 2, PR, 128), BF16), z=((H // 2, 128, 128), F32),
        vt=((4, PR, T), BF16), ot=((2, 2, 128, 128), F32),
        xsel=((8, D), F32), gu=((2, 2, 2, 8, 128), F32), h=((2, 8, 128), F32), y=((8, D), F32), sfix=((16, D), F32))
    work.update({'m%d' % k: ((NPROD, 128, 128), F32) for k in range(4)})
    work.update({'phi%d' % k: ((4, T // 2, 128), U32) for k in range(NU)})
    work.update(xs=((NTILE, NPROD, HT, HD), BF16), wos=((NU, NPROD, HD // 2, 128), U32))
    work.update({'os%d' % k: ((NPROD, HT // 2, HD), U32) for k in range(2)})
    hbm = pl.BlockSpec(memory_space=pl.ANY)
    out = pl.pallas_call(
        _kernel,
        in_specs=[hbm] * 8,
        out_specs=hbm,
        out_shape=jax.ShapeDtypeStruct((S, D), BF16),
        scratch_shapes=[
            pltpu.VMEM((S, D), BF16),
            pltpu.VMEM((D, 3 * D), BF16),
            pltpu.VMEM((D, DH), BF16),
            pltpu.VMEM((8, 128), BF16),
            pltpu.VMEM((D, D), BF16),
            pltpu.VMEM((D, FF), BF16),
            pltpu.VMEM((D, FF), BF16),
            pltpu.VMEM((FF, D), BF16),
            pltpu.VMEM((S, D), BF16),
            pltpu.VMEM((16, D), BF16),
            {k: pltpu.VMEM(shape, dt) for k, (shape, dt) in work.items()},
            pltpu.SemaphoreType.DMA((6,)),
        ],
        compiler_params=pltpu.CompilerParams(vmem_limit_bytes=110 * 2**20),
    )(A_x.reshape(S, D), A_wqkv, A_w_phi.reshape(D, DH), A_wo, B_w_r.reshape(8, 128),
      B_w_gate, B_w_up, B_w_down)
    return out.reshape(1, S, D)


def make(**kw):
    CFG.update(kw)
    return _call


@jax.jit
def pallas_recurrent_scan__linear_kernel_hedgehog__moe_arch_mod__prompt_kernel(
        A_x, A_wqkv, A_w_phi, A_wo, B_x, B_w_r, B_w_gate, B_w_up, B_w_down):
    return make()(A_x, A_wqkv, A_w_phi, A_wo, B_x, B_w_r, B_w_gate, B_w_up, B_w_down)
```

```python
import functools

import jax
import jax.numpy as jnp
from jax import lax
import jax.experimental.pallas as pl
import jax.experimental.pallas.tpu as pltpu

F32 = jnp.float32
BF16 = jnp.bfloat16
U32 = jnp.uint32
LOG2E = 1.4426950408889634
NN = (((1,), (0,)), ((), ()))
NT = (((1,), (1,)), ((), ()))

S, D, H, FF = 2048, 1024, 32, 3584
DH = D // H
HD = D // 2
PR = 2 * DH
NU = 4
UW = D // NU
T = 256
HT = T // 2
NTILE = S // T
NPROD = 7
NORDER = 1024
PAIRS = (2, 3, 0, 1)
P = functools.partial
CFG = dict(ln=4, l1=4, lt=3, fq=2, fk=3, fv=4, wo=3, phi=3, epi=2, vp=1, ot=2, kf=3, ln_k=10, ln_pad=4, gap=3,
           lnc=(4, 8), pin='m z kv phi vt wt wos os fold', wo_n=0, late=0, kv7=5, kvn=0, fw=1, fs=0, ks=6, fsplit=0, fdl=0, plain=[(7, u) for u in range(4)], hq=0, hk=(3,4,5,6,7), wh=6, e0=0, xf=0, fqk=0)


def _dot(a, b, dims=NN):
    return lax.dot_general(a, b, dims, preferred_element_type=F32)


def _bf16_round(v):
    return v.astype(BF16).astype(F32)


def _recip(v):
    return pltpu.reciprocal(v, approx=True)


def _transposed_words(v):
    return pltpu.bitcast(v.astype(BF16).T, U32)


def _pair_reduce(r, op):
    r = op(r, pltpu.roll(r, 4, 0))
    return op(r, pltpu.roll(r, 2, 0))


def _dual_exp(p):
    p3 = p.reshape(8, 8, 128)
    top = _pair_reduce(jnp.max(p3, axis=0), jnp.maximum)
    low = _pair_reduce(jnp.min(p3, axis=0), jnp.minimum)
    e_pos = jnp.exp2(p3 - top[None])
    e_neg = jnp.exp2(low[None] - p3)
    r_pos = _recip(_pair_reduce(jnp.sum(e_pos, axis=0), jnp.add))
    r_neg = _recip(_pair_reduce(jnp.sum(e_neg, axis=0), jnp.add))
    return e_pos, e_neg, r_pos, r_neg


def _features(e_pos, e_neg, r_pos, r_neg):
    return jnp.concatenate([(e_pos * r_pos[None]).reshape(PR, 128), (e_neg * r_neg[None]).reshape(PR, 128)], axis=0)


def _lhs_term(k, a):
    return (lambda: a(0, 0) + a(1, 1), lambda: a(1, 0) + a(1, 1), lambda: a(0, 0), lambda: a(1, 1),
            lambda: a(0, 0) + a(0, 1), lambda: a(1, 0) - a(0, 0), lambda: a(0, 1) - a(1, 1))[k]()


def _rhs_term(k, b):
    return (lambda: b(0, 0) + b(1, 1), lambda: b(0, 0), lambda: b(0, 1) - b(1, 1), lambda: b(1, 0) - b(0, 0),
            lambda: b(1, 1), lambda: b(0, 0) + b(0, 1), lambda: b(1, 0) + b(1, 1))[k]()


def _quadrant(m, i, j):
    if (i, j) == (0, 0):
        return m(0) + m(3) - m(4) + m(6)
    if (i, j) == (0, 1):
        return m(2) + m(4)
    if (i, j) == (1, 0):
        return m(1) + m(3)
    return m(0) - m(1) + m(2) + m(5)


def _layernorm(xf):
    mean = jnp.sum(xf, axis=1, keepdims=True) * (1.0 / D)
    cen = xf - mean
    var = jnp.sum(cen * cen, axis=1, keepdims=True) * (1.0 / D)
    den = _bf16_round(jnp.sqrt(_bf16_round(_bf16_round(var) + 1e-5)))
    return (xf - _bf16_round(mean)) * _recip(den)


def _gated(xf, b, s):
    return xf + s * (b * _recip(1.0 + jnp.exp2(b * (-LOG2E))))


def _touch(*arrays):
    words = [a if a.dtype == U32 else pltpu.bitcast(a, U32) for a in arrays]
    tiles = [w[r:r + 8, c:c + 128] for w in words for r in range(0, w.shape[0], 8) for c in range(0, w.shape[1], 128)]
    return functools.reduce(jnp.bitwise_or, tiles)


def _spread(tasks, lo=0, hi=NPROD, slots=NPROD):
    n = hi - lo
    return [[]] * lo + [tasks[s * len(tasks) // n:(s + 1) * len(tasks) // n] for s in range(n)] + [[]] * (slots - hi)


def _join(*plans):
    return [sum(groups, []) for groups in zip(*plans)]


def _merge(*lists):
    keyed = [((k + 0.5) / len(l), n, t) for n, l in enumerate(lists) for k, t in enumerate(l)]
    return [t for _, _, t in sorted(keyed, key=lambda e: e[:2])]


def _kernel(x_hbm, wqkv_hbm, wphi_hbm, wo_hbm, wr_hbm, wg_hbm, wu_hbm, wd_hbm, out_hbm,
            x_v, w_v, wphi_v, wr_v, wo_v, wg_v, wu_v, wd_v, out_v, fix_v, work, sems):
    bd_v, fold_v, wt_v, xn_v, score_v, best_v, bidx_v = [work[k] for k in 'bd fold wt xn score best bidx'.split()]
    vt_v, kv_v, kvt_v, z_v, ot_v = [work[k] for k in 'vt kv kvt z ot'.split()]
    xsel_v, gu_v, h_v, y_v, sfix_v = [work[k] for k in 'xsel gu h y sfix'.split()]
    xs_v, wos_v = work['xs'], work['wos']
    phi_v = [work['phi%d' % k] for k in range(NU)]
    m_v = [work['m%d' % k] for k in range(4)]
    os_v = [work['os%d' % k] for k in range(2)]

    def copy(src, dst, sem):
        return pltpu.make_async_copy(src, dst, sems.at[sem])

    def x_copy(r0, n, sem):
        return copy(x_hbm.at[pl.ds(r0, n)], x_v.at[pl.ds(r0, n)], sem)

    def w_copy(c0, n, sem):
        return copy(wqkv_hbm.at[:, pl.ds(c0, n)], w_v.at[:, pl.ds(c0, n)], sem)

    def k_copies(u):
        rows = pl.ds(UW, D - UW) if u else pl.ds(0, UW)
        phi = [copy(wphi_hbm.at[rows], wphi_v.at[rows], (u + 2) % 4)] if u < 2 else []
        return [w_copy(D + u * UW, UW, (u + 2) % 4)] + phi

    def v_copy(u):
        return w_copy(2 * D + u * UW, UW, (u + 2) % 4)

    def out_copy(j, u=None, t=None):
        rows = pl.ds(j * T, T) if t is None else pl.ds(j * T + t * HT, HT)
        cols = pl.ds(0, D) if u is None else pl.ds(u * UW, UW)
        return copy(out_v.at[rows, cols], out_hbm.at[rows, cols], 4 if j < NTILE - 1 else 5)

    def sync(starts, waits):
        for cp in starts:
            cp.start()
        for cp in waits:
            cp.wait()

    wr_cp = copy(wr_hbm, wr_v, 0)
    x0_cps = [x_copy(0, HT, 1), x_copy(HT, HT, 4)]
    x1_cp, x23_cp = x_copy(T, T, 4), x_copy(2 * T, 2 * T, 2)
    later_cps = [x_copy(4 * T, S - 4 * T, 3), w_copy(0, D, 3), copy(wo_hbm, wo_v, 3)]
    ffn_cps = [copy(wg_hbm, wg_v, 0), copy(wu_hbm, wu_v, 0), copy(wd_hbm, wd_v, 0)]

    sync([wr_cp] + x0_cps, [wr_cp])
    wr8 = wr_v[...].astype(F32)
    wr_rows = jnp.concatenate([jnp.broadcast_to(wr8[c:c + 1], (8, 128)) for c in range(8)], axis=1)

    order_v = work['order'].at[jnp.where(wr8 > jnp.inf, 1, 0)[0, 0]]
    count = [0]
    due = []

    def after(v):
        k = count[0] % NORDER
        count[0] += 1
        order_v[k] = v
        order_v[k] = jnp.zeros((8, 128), U32)
        return order_v[k]

    def finish_within(products, v):
        due.append([products, after(v)])

    def run(tasks):
        for task in tasks:
            task(None)

    def products(slot, lhs, rhs, dims, plan, jobs):
        for k in range(NPROD):
            for d in due:
                d[0] -= 1
            ready = [d[1] for d in due if d[0] <= 0]
            due[:] = [d for d in due if d[0] > 0]
            words = lhs(k)
            if ready:
                zero = functools.reduce(jnp.bitwise_or, ready)
                last = jnp.concatenate([words[-8:, :-128], words[-8:, -128:] | zero], axis=1)
                words = jnp.concatenate([words[:-8], last], axis=0)
            res = _dot(pltpu.bitcast(words, BF16), rhs(k), dims)
            m_v[slot][k] = res
            if plan[k]:
                begun = pltpu.bitcast(after(pltpu.bitcast(res[0:8], U32)), F32)
                for task in plan[k]:
                    done = task(begun)
                    if done is not None:
                        finish_within(*done)
            for job in jobs.get(k, ()):
                job()

    def block(slot, i, j, rows):
        return _quadrant(lambda k: m_v[slot][k, rows, :], i, j)

    def pair_block(slot, q, t):
        return block(slot, q // 2, t, slice((q % 2) * PR, (q % 2 + 1) * PR))

    def held(v, begun):
        return v if begun is None else v + jnp.tile(begun, (v.shape[0] // 8, v.shape[1] // 128))

    idle = [lambda begun: None]

    def prep_phi(lo, hi):
        r_i = lax.broadcasted_iota(jnp.int32, (128, DH), 0)
        c_i = lax.broadcasted_iota(jnp.int32, (128, DH), 1)
        rep = _dot(((r_i % PR) // 2 == c_i).astype(BF16), wphi_v[lo:hi], NT)
        r_i = lax.broadcasted_iota(jnp.int32, rep.shape, 0)
        c_i = lax.broadcasted_iota(jnp.int32, rep.shape, 1)
        bd_v[:, lo:hi] = jnp.where((r_i // PR) * 2 + r_i % 2 == (c_i % 128) // DH, rep, 0.0).astype(BF16)

    def fold(m, u):
        for g in range(2):
            c0 = u * UW + g * 128
            fold_v[u, g] = _dot(bd_v[:, c0:c0 + 128], w_v[:, m * D + c0:m * D + c0 + 128], NT) * LOG2E

    def proj_terms(m, u, c, ks, begun):
        cols = lambda h: slice(h * HD + c * 128, h * HD + (c + 1) * 128)
        if m < 2 and CFG['xf']:
            outs = [_transposed_words(_lhs_term(k, lambda g, h: fold_v[u, g, :, cols(h)].T)) for k in ks]
        elif m < 2:
            outs = [pltpu.bitcast(_lhs_term(k, lambda g, h: fold_v[u, g, :, cols(h)]).astype(BF16), U32) for k in ks]
        else:
            c0 = 2 * D + u * UW
            blk = lambda g, h: w_v[cols(h), c0 + g * 128:c0 + (g + 1) * 128].astype(F32)
            outs = [_transposed_words(_lhs_term(k, blk)) for k in ks]
        for k, words in zip(ks, outs):
            wt_v[m, u, k, :, c * 128:(c + 1) * 128] = words
        return CFG['fv' if m == 2 else 'fk' if m else 'fq'], _touch(*outs)

    def weight_tasks(m, u):
        return [P(proj_terms, m, u, c, ks) for ks in ((0, 1, 2), (3, 4), (5, 6)) for c in range(4)]

    def wo_terms(u, g, ks, begun):
        blk = lambda i, j: wo_v[g * UW + i * 128:g * UW + (i + 1) * 128,
                                u * UW + j * 128:u * UW + (j + 1) * 128].astype(F32)
        outs = [pltpu.bitcast(_rhs_term(k, blk).astype(BF16), U32) for k in ks]
        for k, words in zip(ks, outs):
            wos_v[u, k, g * 64:(g + 1) * 64, :] = words
        return CFG['wo'], _touch(*outs)

    def ln_norm(g, begun):
        xn = _layernorm(x_v[g * 8:(g + 1) * 8, :].astype(F32))
        xn_v[g * 8:(g + 1) * 8, :] = xn.astype(BF16)
        r = jnp.broadcast_to(_bf16_round(jnp.sum(xn * held(wr_rows, begun), axis=1, keepdims=True)), (8, 128))
        score_v[g] = r
        return CFG['ln' if g >= 64 else 'l1'], _touch(xn, r)

    def ln_best(i, begun):
        best = jnp.full((8, 128), -jnp.inf, F32)
        first = jnp.full((8, 128), S, jnp.int32)
        for g in range(i * T // 8, (i + 1) * T // 8):
            r = score_v[g]
            tok = lax.broadcasted_iota(jnp.int32, (8, 128), 0) + g * 8
            take = (r > best) | ((r == best) & (tok < first))
            best, first = jnp.where(take, r, best), jnp.where(take, tok, first)
        best_v[i], bidx_v[i] = best, first
        return CFG['ln'], _touch(best, first)

    x_ops = {}

    def ln_terms(i, c, begun):
        blk = lambda h, t: xn_v[i * T + t * HT + c * 16:i * T + t * HT + (c + 1) * 16, h * HD:(h + 1) * HD].astype(F32)
        outs = {k: _rhs_term(k, blk) for k in (0, 2, 3, 5, 6)}
        for k, term in outs.items():
            xs_v[i, k, c * 16:(c + 1) * 16, :] = term.astype(BF16)
        return CFG['lt'], _touch(*outs.values())

    def x_operand(i, k):
        if (i, k) not in x_ops:
            if k in (1, 4):
                t = k // 4
                x_ops[i, k] = xn_v[i * T + t * HT:i * T + (t + 1) * HT, t * HD:(t + 1) * HD]
            else:
                x_ops[i, k] = xs_v[i, k]
        return x_ops[i, k]

    def ln_tasks(i):
        norm = lambda c: [P(ln_norm, (i * T + t * HT + c * 16) // 8 + e) for t in range(2) for e in range(2)]
        tasks = norm(0)
        for c in range(1, HT // 16):
            tasks += norm(c)[:3] + [P(ln_terms, i, c - 1)] + norm(c)[3:]
        return tasks + idle * CFG['gap'] + [P(ln_terms, i, HT // 16 - 1), P(ln_best, i)]

    def proj(m, u, i, slot, plan, jobs=None):
        products(slot, lambda k: wt_v[m, u, k], lambda k: x_operand(i, k), NT, plan, jobs or {})

    def keep_features(u, q, n, f):
        words = _transposed_words(f)
        phi_v[u][q, n * 64:(n + 1) * 64, :] = words
        return words

    def phi_k(i, u, slot, q, t, begun):
        f = _features(*_dual_exp(held(pair_block(slot, q, t), begun if i in CFG['hk'] else None)))
        words = keep_features(u, q, i % 2 * 2 + t, f)
        z = f + z_v[u * 4 + q] if i or t else f
        z_v[u * 4 + q] = z
        return CFG['phi'], _touch(z, words)

    def v_round(i, u, slot, q, begun):
        v = jnp.concatenate([pair_block(slot, q, t) for t in range(2)], axis=1)
        vt_v[u, q, :, i % 2 * T:(i % 2 + 1) * T] = v.astype(BF16)
        return CFG['vp'], _touch(v)

    def kv_update(i, u):
        if i % 2 == 0:
            return
        for q in PAIRS:
            acc = _dot(vt_v[u, q], pltpu.bitcast(phi_v[u][q], BF16))
            if i > 1:
                acc = acc + kv_v[u * 4 + q]
            kv_v[u * 4 + q] = acc
            finish_within(3, _touch(acc))

    def kv_finish(p, begun):
        r_i = lax.broadcasted_iota(jnp.int32, (PR, 128), 0)
        c_i = lax.broadcasted_iota(jnp.int32, (PR, 128), 1)
        z = jnp.broadcast_to(jnp.sum(z_v[p], axis=1, keepdims=True), (128, 128))
        z_v[p] = z
        kvt_v[p] = jnp.where(r_i // DH == c_i % 2, kv_v[p], 0.0).astype(BF16)
        return CFG['kf'], _touch(z)

    def key_tasks(i, u, slot):
        return [P(phi_k, i, u, slot, q, t) for q in PAIRS for t in range(2)]

    def value_tasks(i, u, slot):
        return [P(v_round, i, u, slot, q) for q in PAIRS]

    sync(k_copies(0), x0_cps[:1])
    sync(k_copies(1), x0_cps[1:])
    run(ln_tasks(0))
    sync(k_copies(2), k_copies(0))
    prep_phi(0, UW)
    fold(1, 0)
    run(weight_tasks(1, 0))
    starts = [k_copies(3), [v_copy(0)], [v_copy(1), x1_cp], [v_copy(2)]]
    for u in range(NU):
        a = 2 if u else 3
        if u + 1 < NU:
            job = [P(sync, starts[u], k_copies(u + 1))] + ([] if u else [P(prep_phi, UW, D)]) + [P(fold, 1, u + 1)]
            late = weight_tasks(1, u + 1)
        else:
            job = [P(sync, starts[u], [v_copy(0)])]
            late = weight_tasks(2, 0)
        early = key_tasks(0, u - 1, 2 + (u - 1) % 2) if u else []
        proj(1, u, 0, 2 + u % 2, _join(_spread(early, 0, a + 1), _spread(late, a + 1)), {a: job})
    starts = [[v_copy(3)], [x23_cp], later_cps]
    waits = [[v_copy(1), x1_cp], [v_copy(2)], [v_copy(3)]]
    ln = ln_tasks(1)
    c0, c1 = [len(ln) * f // 16 for f in CFG['lnc']]
    ln = _join(_spread(ln[:c0], 3, 7, 28), _spread(ln[c0:c1], 10, 14, 28), _spread(ln[c1:], 17, 25, 28))
    for u in range(NU):
        early = value_tasks(0, u - 1, (u - 1) % 2) if u else key_tasks(0, NU - 1, 3)
        jobs = {NPROD - 1: [P(kv_update, 0, u - 1)]} if u else {}
        plan = _spread(early)
        if u + 1 < NU:
            jobs[2] = [P(sync, starts[u], waits[u])]
            plan = _join(_spread(early, 0, 3), _spread(weight_tasks(2, u + 1), 3))
        proj(2, u, 0, u % 2, _join(plan, ln[NPROD * u:NPROD * (u + 1)]), jobs)

    wo_tasks = [P(wo_terms, u, g, ks) for u in range(NU) for g in range(NU) for ks in ((0, 1, 2), (3, 4, 5, 6))]
    prev = (0, NU - 1)
    for i in range(1, NTILE):
        if i == 1:
            sync([], [x23_cp])
        if i == 3:
            sync(ffn_cps, later_cps)
        side = ln_tasks(i + 1) + idle * CFG['ln_pad'] if i + 1 < NTILE else wo_tasks[4 * CFG['wo_n']:]
        for u in range(NU):
            mine = side[u * len(side) // NU:(u + 1) * len(side) // NU]
            cut = len(mine) * CFG['ln_k'] // 14 if i + 1 < NTILE else len(mine)
            k_tasks = _merge(value_tasks(*prev, 1), mine[:cut])
            v_tasks = _merge(key_tasks(i, u, 0), mine[cut:])
            k_jobs = {CFG['ks']: [P(kv_update, *prev)]}
            if 3 <= i < 3 + NU:
                if u == 0:
                    k_jobs[0] = [P(fold, 0, i - 3)]
                k_tasks = _merge(k_tasks, weight_tasks(0, i - 3)[3 * u:3 * u + 3]) if CFG['fqk'] and u else k_tasks
                v_tasks = v_tasks if CFG['fqk'] and u else _merge(v_tasks, weight_tasks(0, i - 3)[3 * u:3 * u + 3])
                n = CFG['wo_n']
                k_tasks = _merge(k_tasks, wo_tasks[(i - 3) * n + u * n // NU:(i - 3) * n + (u + 1) * n // NU])
            if i == NTILE - 1 and u > 1:
                k_tasks = _merge(k_tasks, [P(kv_finish, (u - 2) * 4 + q) for q in range(4)])
            proj(1, u, i, 0, _spread(k_tasks), k_jobs)
            proj(2, u, i, 1, _spread(v_tasks))
            prev = (i, u)

    best = jnp.max(jnp.max(best_v[...], axis=0), axis=0, keepdims=True)
    first = jnp.min(jnp.min(jnp.where(best_v[...] == best[None], bidx_v[...], S), axis=0), axis=0, keepdims=True)
    idx = jnp.where(first[0, 0] == S, 0, first[0, 0])
    route_gate = _bf16_round(jax.nn.sigmoid(jnp.where(first == S, jnp.nan, best)))[:, 0:1]
    fix_grp = jnp.where(idx >= S - T, 0, idx // 16)
    fix_rows = pl.ds(pl.multiple_of(fix_grp * 16, 16), 16)
    fix_cp = copy(fix_v, out_hbm.at[fix_rows], 5)

    def ffn_input(begun):
        xsel = _bf16_round(_layernorm(x_v[pl.ds(pl.multiple_of((idx // 8) * 8, 8), 8), :].astype(F32)))
        xsel_v[...] = xsel
        sfix_v[...] = jnp.zeros(sfix_v.shape, F32)
        return 5, _touch(xsel)

    def ffn_up(c, which, h):
        half = slice(h * HD, (h + 1) * HD)
        gu_v[c % 2, which, h] = _dot(xsel_v[:, half], (wg_v, wu_v)[which][half, c * 128:(c + 1) * 128])
        if which and h:
            g = gu_v[c % 2, 0, 0] + gu_v[c % 2, 0, 1]
            h_v[c % 2] = _bf16_round(g * jax.nn.sigmoid(g) * (gu_v[c % 2, 1, 0] + gu_v[c % 2, 1, 1]))

    def ffn_down(c, h):
        half = slice(h * HD, (h + 1) * HD)
        y = _dot(h_v[c % 2], wd_v[c * 128:(c + 1) * 128, half])
        if c:
            y = y + y_v[:, half]
        y_v[:, half] = y
        finish_within(3, _touch(y))

    ffn = []
    for c in range(FF // 128):
        ffn += [P(ffn_up, c, which, h) for which in range(2) for h in range(2)]
        ffn += [P(ffn_down, c - 1, h) for h in range(2)] if c else []
    ffn += [P(ffn_down, FF // 128 - 1, h) for h in range(2)]

    def routed_update(cols):
        y = y_v[:, cols]
        mine = lax.broadcasted_iota(jnp.int32, y.shape, 0) == idx % 8
        return _bf16_round(_bf16_round(jnp.sum(jnp.where(mine, y, 0.0), axis=0, keepdims=True)) * route_gate)

    def fix_routed():
        b = xn_v[fix_rows, :].astype(F32)
        row = lax.broadcasted_iota(jnp.int32, b.shape, 0) + fix_grp * 16
        b = jnp.where(row == idx, _bf16_round(b + routed_update(slice(None))), b)
        fix_v[...] = _gated(x_v[fix_rows, :].astype(F32), b, sfix_v[...]).astype(BF16)

    def phi_q(u, slot, q, t, hold, begun):
        e_pos, e_neg, r_pos, r_neg = _dual_exp(held(pair_block(slot, q, t), begun if hold else None))
        a = jnp.sum(e_pos * z_v[u * 4 + q, :PR].reshape(8, 8, 128), axis=0)
        b = jnp.sum(e_neg * z_v[u * 4 + q, PR:].reshape(8, 8, 128), axis=0)
        r_den = _recip(_pair_reduce(r_pos * a + r_neg * b, jnp.add) + 1e-6)
        f = _features(e_pos, e_neg, r_pos * r_den, r_neg * r_den)
        return CFG['phi'], _touch(keep_features(u, q, t, f))

    def attend(u):
        for q in PAIRS:
            o = _dot(kvt_v[u * 4 + q], pltpu.bitcast(phi_v[u][q, :T // 2], BF16), NT)
            for t in range(2):
                ot_v[q // 2, t, (q % 2) * PR:(q % 2 + 1) * PR, :] = o[:, t * 128:(t + 1) * 128]

    def o_terms(j, u, ks, begun):
        outs = [_transposed_words(_lhs_term(k, lambda t, g: ot_v[g, t])) for k in ks]
        for k, words in zip(ks, outs):
            os_v[j % 2][k, :, u * 128:(u + 1) * 128] = words
        return CFG['ot'], _touch(*outs)

    def out_proj(j, u, slot, plan):
        products(slot, lambda k: os_v[j % 2][k], lambda k: pltpu.bitcast(wos_v[u, k], BF16), NN, plan, {})

    def epilogue(j, u, slot, t, c, begun):
        r0 = j * T + t * HT + c * 64
        cols = slice(u * UW, (u + 1) * UW)
        s = jnp.concatenate([block(slot, t, h, slice(c * 64, (c + 1) * 64)) for h in range(2)], axis=1)
        b = xn_v[r0:r0 + 64, cols].astype(F32)
        kept = []
        if j == NTILE - 1:
            row = lax.broadcasted_iota(jnp.int32, b.shape, 0) + r0
            b = jnp.where(row == idx, _bf16_round(b + routed_update(cols)), b)
        else:
            keep = sfix_v[:, cols]
            for g in range(4):
                keep = jnp.where(fix_grp == r0 // 16 + g, s[g * 16:(g + 1) * 16], keep)
            sfix_v[:, cols] = keep
            kept = [keep]
        res = _gated(x_v[r0:r0 + 64, cols].astype(F32), b, s)
        out_v[r0:r0 + 64, cols] = res.astype(BF16)
        return CFG['epi'], _touch(res, *kept)

    steps = [(j, u) for j in range(NTILE) for u in range(NU)]
    lag = NU + 1
    waiting = []
    for n in range(len(steps) + lag + 1):
        cur = steps[n] if n < len(steps) else None
        att = steps[n - 1] if 1 <= n <= len(steps) else None
        out = steps[n - lag] if lag <= n < len(steps) + lag else None
        epi = steps[n - lag - 1] if n > lag else None
        ends = [P(epilogue, *epi, 2 + (n - 1) % 2, t, c) for t in (1, 0) for c in range(2)] if epi else []
        soft = [P(phi_q, cur[1], n % 2, q, t, n < CFG['hq']) for q in PAIRS for t in range(2)] if cur else []
        terms = [P(o_terms, *att, ks) for ks in ((0, 1), (2, 3, 4), (5, 6))] if att else []
        if n == CFG['fw']:
            sync([], ffn_cps)
        if n == 0:
            plan = _join(_spread(value_tasks(*prev, 1), 0, 3), _spread([P(kv_finish, 8 + q) for q in range(4)], 3))
            proj(0, cur[1], cur[0], 0, plan, {CFG['kv7']: [P(kv_update, *prev)]} if CFG['kvn'] == 0 else {})
            waiting = [ffn_input] + soft
        elif not out and cur:
            proj(0, cur[1], cur[0], n % 2, _spread(waiting, 0, CFG['wh']),
                 {CFG['kv7']: [P(kv_update, *prev)]} if n == CFG['kvn'] else {})
            attend(att[1])
            waiting = _merge(terms, soft) + ([P(kv_finish, 12 + q) for q in range(4)] if n == 2 else [])
        elif cur:
            jobs = {k: [job] for k, job in enumerate(ffn[(n - lag) * NPROD:(n - lag + 1) * NPROD])}
            proj(0, cur[1], cur[0], n % 2, _join(_spread(waiting, 0, 5), _spread(ends, CFG['e0'])), jobs)
            waiting = terms if CFG['late'] and cur != steps[-1] else []
            attend(att[1])
            if epi and epi[1] == NU - 1:
                out_copy(epi[0]).start()
            out_proj(*out, 2 + n % 2, _spread(soft if waiting else terms + soft))
        elif out:
            if att:
                attend(att[1])
            out_proj(*out, 2 + n % 2, _spread(_merge(terms, ends)))
            if epi == (NTILE - 2, NU - 1):
                out_copy(epi[0]).start()
            if epi[0] == NTILE - 1:
                out_copy(*epi).start()
            if epi == (NTILE - 1, 0):
                sync([], [out_copy(j) for j in range(NTILE - 1)])
                fix_routed()
                fix_cp.start()
        else:
            for k, t in enumerate((1, 0)):
                run(ends[2 * k:2 * k + 2])
                out_copy(*epi, t).start()

    pins = [r for k, r in work.items() if k.rstrip('0123') in CFG['pin'].split()]
    pins = [copy(r.at[(0,) * (len(r.shape) - 2) + (pl.ds(0, 8), pl.ds(0, 128))], work[r.dtype.name].at[k], 5)
            for k, r in enumerate(pins)]
    sync(pins, pins + [fix_cp] + [out_copy(NTILE - 1, u) for u in range(NU - 1)]
         + [out_copy(NTILE - 1, NU - 1, t) for t in range(2)])


def _call(A_x, A_wqkv, A_w_phi, A_wo, B_x, B_w_r, B_w_gate, B_w_up, B_w_down):
    del B_x
    work = dict(
        order=((1, NORDER, 8, 128), U32), float32=((16, 8, 128), F32), uint32=((16, 8, 128), U32),
        bfloat16=((16, 8, 128), BF16),
        bd=((128, D), BF16), fold=((NU, 2, 128, D), F32), wt=((3, NU, NPROD, 64, HD), U32),
        xn=((S, D), BF16), score=((S // 8, 8, 128), F32),
        best=((NTILE, 8, 128), F32), bidx=((NTILE, 8, 128), jnp.int32),
        kv=((H // 2, PR, 128), F32), kvt=((H // 2, PR, 128), BF16), z=((H // 2, 128, 128), F32),
        vt=((NU, 4, PR, 2 * T), BF16), ot=((2, 2, 128, 128), F32),
        xsel=((8, D), F32), gu=((2, 2, 2, 8, 128), F32), h=((2, 8, 128), F32), y=((8, D), F32), sfix=((16, D), F32))
    work.update({'m%d' % k: ((NPROD, 128, 128), F32) for k in range(4)})
    work.update({'phi%d' % k: ((4, T, 128), U32) for k in range(NU)})
    work.update(xs=((NTILE, NPROD, HT, HD), BF16), wos=((NU, NPROD, HD // 2, 128), U32))
    work.update({'os%d' % k: ((NPROD, HT // 2, HD), U32) for k in range(2)})
    hbm = pl.BlockSpec(memory_space=pl.ANY)
    out = pl.pallas_call(
        _kernel,
        in_specs=[hbm] * 8,
        out_specs=hbm,
        out_shape=jax.ShapeDtypeStruct((S, D), BF16),
        scratch_shapes=[
            pltpu.VMEM((S, D), BF16),
            pltpu.VMEM((D, 3 * D), BF16),
            pltpu.VMEM((D, DH), BF16),
            pltpu.VMEM((8, 128), BF16),
            pltpu.VMEM((D, D), BF16),
            pltpu.VMEM((D, FF), BF16),
            pltpu.VMEM((D, FF), BF16),
            pltpu.VMEM((FF, D), BF16),
            pltpu.VMEM((S, D), BF16),
            pltpu.VMEM((16, D), BF16),
            {k: pltpu.VMEM(shape, dt) for k, (shape, dt) in work.items()},
            pltpu.SemaphoreType.DMA((6,)),
        ],
        compiler_params=pltpu.CompilerParams(vmem_limit_bytes=110 * 2**20),
    )(A_x.reshape(S, D), A_wqkv, A_w_phi.reshape(D, DH), A_wo, B_w_r.reshape(8, 128),
      B_w_gate, B_w_up, B_w_down)
    return out.reshape(1, S, D)


def make(**kw):
    CFG.update(kw)
    return _call


@jax.jit
def pallas_recurrent_scan__linear_kernel_hedgehog__moe_arch_mod__prompt_kernel(
        A_x, A_wqkv, A_w_phi, A_wo, B_x, B_w_r, B_w_gate, B_w_up, B_w_down):
    return make()(A_x, A_wqkv, A_w_phi, A_wo, B_x, B_w_r, B_w_gate, B_w_up, B_w_down)
```

```python
import functools

import jax
import jax.numpy as jnp
from jax import lax
import jax.experimental.pallas as pl
import jax.experimental.pallas.tpu as pltpu

F32 = jnp.float32
BF16 = jnp.bfloat16
U32 = jnp.uint32
LOG2E = 1.4426950408889634
NN = (((1,), (0,)), ((), ()))
NT = (((1,), (1,)), ((), ()))

S, D, H, FF = 2048, 1024, 32, 3584
DH = D // H
HD = D // 2
PR = 2 * DH
NU = 4
UW = D // NU
T = 256
HT = T // 2
NTILE = S // T
NPROD = 7
NORDER = 1024
PAIRS = (2, 3, 0, 1)
P = functools.partial
PINNED = 'm z kv phi vt wt wos os fold'.split()


def _dot(a, b, dims=NN):
    return lax.dot_general(a, b, dims, preferred_element_type=F32)


def _bf16_round(v):
    return v.astype(BF16).astype(F32)


def _recip(v):
    return pltpu.reciprocal(v, approx=True)


def _transposed_words(v):
    return pltpu.bitcast(v.astype(BF16).T, U32)


def _pair_reduce(r, op):
    r = op(r, pltpu.roll(r, 4, 0))
    return op(r, pltpu.roll(r, 2, 0))


def _dual_exp(p):
    p3 = p.reshape(8, 8, 128)
    top = _pair_reduce(jnp.max(p3, axis=0), jnp.maximum)
    low = _pair_reduce(jnp.min(p3, axis=0), jnp.minimum)
    e_pos = jnp.exp2(p3 - top[None])
    e_neg = jnp.exp2(low[None] - p3)
    r_pos = _recip(_pair_reduce(jnp.sum(e_pos, axis=0), jnp.add))
    r_neg = _recip(_pair_reduce(jnp.sum(e_neg, axis=0), jnp.add))
    return e_pos, e_neg, r_pos, r_neg


def _features(e_pos, e_neg, r_pos, r_neg):
    return jnp.concatenate([(e_pos * r_pos[None]).reshape(PR, 128), (e_neg * r_neg[None]).reshape(PR, 128)], axis=0)


def _lhs_term(k, a):
    return (lambda: a(0, 0) + a(1, 1), lambda: a(1, 0) + a(1, 1), lambda: a(0, 0), lambda: a(1, 1),
            lambda: a(0, 0) + a(0, 1), lambda: a(1, 0) - a(0, 0), lambda: a(0, 1) - a(1, 1))[k]()


def _rhs_term(k, b):
    return (lambda: b(0, 0) + b(1, 1), lambda: b(0, 0), lambda: b(0, 1) - b(1, 1), lambda: b(1, 0) - b(0, 0),
            lambda: b(1, 1), lambda: b(0, 0) + b(0, 1), lambda: b(1, 0) + b(1, 1))[k]()


def _quadrant(m, i, j):
    if (i, j) == (0, 0):
        return m(0) + m(3) - m(4) + m(6)
    if (i, j) == (0, 1):
        return m(2) + m(4)
    if (i, j) == (1, 0):
        return m(1) + m(3)
    return m(0) - m(1) + m(2) + m(5)


def _layernorm(xf):
    mean = jnp.sum(xf, axis=1, keepdims=True) * (1.0 / D)
    cen = xf - mean
    var = jnp.sum(cen * cen, axis=1, keepdims=True) * (1.0 / D)
    den = _bf16_round(jnp.sqrt(_bf16_round(_bf16_round(var) + 1e-5)))
    return (xf - _bf16_round(mean)) * _recip(den)


def _gated(xf, b, s):
    return xf + s * (b * _recip(1.0 + jnp.exp2(b * (-LOG2E))))


def _touch(*arrays):
    words = [a if a.dtype == U32 else pltpu.bitcast(a, U32) for a in arrays]
    tiles = [w[r:r + 8, c:c + 128] for w in words for r in range(0, w.shape[0], 8) for c in range(0, w.shape[1], 128)]
    return functools.reduce(jnp.bitwise_or, tiles)


def _spread(tasks, lo=0, hi=NPROD, slots=NPROD):
    n = hi - lo
    return [[]] * lo + [tasks[s * len(tasks) // n:(s + 1) * len(tasks) // n] for s in range(n)] + [[]] * (slots - hi)


def _join(*plans):
    return [sum(groups, []) for groups in zip(*plans)]


def _merge(*lists):
    keyed = [((k + 0.5) / len(l), n, t) for n, l in enumerate(lists) for k, t in enumerate(l)]
    return [t for _, _, t in sorted(keyed, key=lambda e: e[:2])]


def _kernel(x_hbm, wqkv_hbm, wphi_hbm, wo_hbm, wr_hbm, wg_hbm, wu_hbm, wd_hbm, out_hbm,
            x_v, w_v, wphi_v, wr_v, wo_v, wg_v, wu_v, wd_v, out_v, fix_v, work, sems):
    bd_v, fold_v, wt_v, xn_v, score_v, best_v, bidx_v = [work[k] for k in 'bd fold wt xn score best bidx'.split()]
    vt_v, kv_v, kvt_v, z_v, ot_v = [work[k] for k in 'vt kv kvt z ot'.split()]
    xsel_v, gu_v, h_v, y_v, sfix_v = [work[k] for k in 'xsel gu h y sfix'.split()]
    xs_v, wos_v = work['xs'], work['wos']
    phi_v = [work['phi%d' % k] for k in range(NU)]
    m_v = [work['m%d' % k] for k in range(4)]
    os_v = [work['os%d' % k] for k in range(2)]

    def copy(src, dst, sem):
        return pltpu.make_async_copy(src, dst, sems.at[sem])

    def x_copy(r0, n, sem):
        return copy(x_hbm.at[pl.ds(r0, n)], x_v.at[pl.ds(r0, n)], sem)

    def w_copy(c0, n, sem):
        return copy(wqkv_hbm.at[:, pl.ds(c0, n)], w_v.at[:, pl.ds(c0, n)], sem)

    def k_copies(u):
        rows = pl.ds(UW, D - UW) if u else pl.ds(0, UW)
        phi = [copy(wphi_hbm.at[rows], wphi_v.at[rows], (u + 2) % 4)] if u < 2 else []
        return [w_copy(D + u * UW, UW, (u + 2) % 4)] + phi

    def v_copy(u):
        return w_copy(2 * D + u * UW, UW, (u + 2) % 4)

    def out_copy(j, u=None, t=None):
        rows = pl.ds(j * T, T) if t is None else pl.ds(j * T + t * HT, HT)
        cols = pl.ds(0, D) if u is None else pl.ds(u * UW, UW)
        return copy(out_v.at[rows, cols], out_hbm.at[rows, cols], 4 if j < NTILE - 1 else 5)

    def sync(starts, waits):
        for cp in starts:
            cp.start()
        for cp in waits:
            cp.wait()

    wr_cp = copy(wr_hbm, wr_v, 0)
    x0_cps = [x_copy(0, HT, 1), x_copy(HT, HT, 4)]
    x1_cp, x23_cp = x_copy(T, T, 4), x_copy(2 * T, 2 * T, 2)
    later_cps = [x_copy(4 * T, S - 4 * T, 3), w_copy(0, D, 3), copy(wo_hbm, wo_v, 3)]
    ffn_cps = [copy(wg_hbm, wg_v, 0), copy(wu_hbm, wu_v, 0), copy(wd_hbm, wd_v, 0)]

    sync([wr_cp] + x0_cps, [wr_cp])
    wr8 = wr_v[...].astype(F32)
    wr_rows = jnp.concatenate([jnp.broadcast_to(wr8[c:c + 1], (8, 128)) for c in range(8)], axis=1)

    order_v = work['order'].at[jnp.where(wr8 > jnp.inf, 1, 0)[0, 0]]
    count = [0]
    due = []

    def after(v):
        k = count[0] % NORDER
        count[0] += 1
        order_v[k] = v
        order_v[k] = jnp.zeros((8, 128), U32)
        return order_v[k]

    def finish_within(products, v):
        due.append([products, after(v)])

    def run(tasks):
        for task in tasks:
            task(None)

    def products(slot, lhs, rhs, dims, plan, jobs):
        for k in range(NPROD):
            for d in due:
                d[0] -= 1
            ready = [d[1] for d in due if d[0] <= 0]
            due[:] = [d for d in due if d[0] > 0]
            words = lhs(k)
            if ready:
                zero = functools.reduce(jnp.bitwise_or, ready)
                last = jnp.concatenate([words[-8:, :-128], words[-8:, -128:] | zero], axis=1)
                words = jnp.concatenate([words[:-8], last], axis=0)
            res = _dot(pltpu.bitcast(words, BF16), rhs(k), dims)
            m_v[slot][k] = res
            if plan[k]:
                begun = pltpu.bitcast(after(pltpu.bitcast(res[0:8], U32)), F32)
                for task in plan[k]:
                    done = task(begun)
                    if done is not None:
                        finish_within(*done)
            for job in jobs.get(k, ()):
                job()

    def block(slot, i, j, rows):
        return _quadrant(lambda k: m_v[slot][k, rows, :], i, j)

    def pair_block(slot, q, t):
        return block(slot, q // 2, t, slice((q % 2) * PR, (q % 2 + 1) * PR))

    def held(v, begun):
        return v if begun is None else v + jnp.tile(begun, (v.shape[0] // 8, v.shape[1] // 128))

    idle = [lambda begun: None]

    def prep_phi(lo, hi):
        r_i = lax.broadcasted_iota(jnp.int32, (128, DH), 0)
        c_i = lax.broadcasted_iota(jnp.int32, (128, DH), 1)
        rep = _dot(((r_i % PR) // 2 == c_i).astype(BF16), wphi_v[lo:hi], NT)
        r_i = lax.broadcasted_iota(jnp.int32, rep.shape, 0)
        c_i = lax.broadcasted_iota(jnp.int32, rep.shape, 1)
        bd_v[:, lo:hi] = jnp.where((r_i // PR) * 2 + r_i % 2 == (c_i % 128) // DH, rep, 0.0).astype(BF16)

    def fold(m, u):
        for g in range(2):
            c0 = u * UW + g * 128
            fold_v[u, g] = _dot(bd_v[:, c0:c0 + 128], w_v[:, m * D + c0:m * D + c0 + 128], NT) * LOG2E

    def proj_terms(m, u, c, ks, begun):
        cols = lambda h: slice(h * HD + c * 128, h * HD + (c + 1) * 128)
        if m < 2:
            outs = [pltpu.bitcast(_lhs_term(k, lambda g, h: fold_v[u, g, :, cols(h)]).astype(BF16), U32) for k in ks]
        else:
            c0 = 2 * D + u * UW
            blk = lambda g, h: w_v[cols(h), c0 + g * 128:c0 + (g + 1) * 128].astype(F32)
            outs = [_transposed_words(_lhs_term(k, blk)) for k in ks]
        for k, words in zip(ks, outs):
            wt_v[m, u, k, :, c * 128:(c + 1) * 128] = words
        return (4 if m == 1 else 3), _touch(*outs)

    def weight_tasks(m, u):
        return [P(proj_terms, m, u, c, ks) for ks in ((0, 1, 2), (3, 4), (5, 6)) for c in range(4)]

    def wo_terms(u, g, ks, begun):
        blk = lambda i, j: wo_v[g * UW + i * 128:g * UW + (i + 1) * 128,
                                u * UW + j * 128:u * UW + (j + 1) * 128].astype(F32)
        outs = [pltpu.bitcast(_rhs_term(k, blk).astype(BF16), U32) for k in ks]
        for k, words in zip(ks, outs):
            wos_v[u, k, g * 64:(g + 1) * 64, :] = words
        return 2, _touch(*outs)

    def ln_norm(g, begun):
        xn = _layernorm(x_v[g * 8:(g + 1) * 8, :].astype(F32))
        xn_v[g * 8:(g + 1) * 8, :] = xn.astype(BF16)
        r = jnp.broadcast_to(_bf16_round(jnp.sum(xn * held(wr_rows, begun), axis=1, keepdims=True)), (8, 128))
        score_v[g] = r
        return (4 if g >= 2 * T // 8 else 3), _touch(xn, r)

    def ln_best(i, begun):
        best = jnp.full((8, 128), -jnp.inf, F32)
        first = jnp.full((8, 128), S, jnp.int32)
        for g in range(i * T // 8, (i + 1) * T // 8):
            r = score_v[g]
            tok = lax.broadcasted_iota(jnp.int32, (8, 128), 0) + g * 8
            take = (r > best) | ((r == best) & (tok < first))
            best, first = jnp.where(take, r, best), jnp.where(take, tok, first)
        best_v[i], bidx_v[i] = best, first
        return 4, _touch(best, first)

    x_ops = {}

    def ln_terms(i, c, begun):
        blk = lambda h, t: xn_v[i * T + t * HT + c * 16:i * T + t * HT + (c + 1) * 16, h * HD:(h + 1) * HD].astype(F32)
        outs = {k: _rhs_term(k, blk) for k in (0, 2, 3, 5, 6)}
        for k, term in outs.items():
            xs_v[i, k, c * 16:(c + 1) * 16, :] = term.astype(BF16)
        return 4, _touch(*outs.values())

    def x_operand(i, k):
        if (i, k) not in x_ops:
            if k in (1, 4):
                t = k // 4
                x_ops[i, k] = xn_v[i * T + t * HT:i * T + (t + 1) * HT, t * HD:(t + 1) * HD]
            else:
                x_ops[i, k] = xs_v[i, k]
        return x_ops[i, k]

    def ln_tasks(i):
        norm = lambda c: [P(ln_norm, (i * T + t * HT + c * 16) // 8 + e) for t in range(2) for e in range(2)]
        tasks = norm(0)
        for c in range(1, HT // 16):
            tasks += norm(c)[:3] + [P(ln_terms, i, c - 1)] + norm(c)[3:]
        return tasks + idle * 3 + [P(ln_terms, i, HT // 16 - 1), P(ln_best, i)]

    def proj(m, u, i, slot, plan, jobs=None):
        products(slot, lambda k: wt_v[m, u, k], lambda k: x_operand(i, k), NT, plan, jobs or {})

    def keep_features(u, q, n, f):
        words = _transposed_words(f)
        phi_v[u][q, n * 64:(n + 1) * 64, :] = words
        return words

    def phi_k(i, u, slot, q, t, begun):
        f = _features(*_dual_exp(held(pair_block(slot, q, t), begun if i else None)))
        words = keep_features(u, q, i % 2 * 2 + t, f)
        z = f + z_v[u * 4 + q] if i or t else f
        z_v[u * 4 + q] = z
        return 5, _touch(z, words)

    def v_round(i, u, slot, q, begun):
        v = jnp.concatenate([pair_block(slot, q, t) for t in range(2)], axis=1)
        vt_v[u, q, :, i % 2 * T:(i % 2 + 1) * T] = v.astype(BF16)
        return 1, _touch(v)

    def kv_update(i, u):
        if i % 2 == 0:
            return
        for q in PAIRS:
            acc = _dot(vt_v[u, q], pltpu.bitcast(phi_v[u][q], BF16))
            if i > 1:
                acc = acc + kv_v[u * 4 + q]
            kv_v[u * 4 + q] = acc
            finish_within(3, _touch(acc))

    def kv_finish(p, begun):
        r_i = lax.broadcasted_iota(jnp.int32, (PR, 128), 0)
        c_i = lax.broadcasted_iota(jnp.int32, (PR, 128), 1)
        z = jnp.broadcast_to(jnp.sum(z_v[p], axis=1, keepdims=True), (128, 128))
        z_v[p] = z
        kvt_v[p] = jnp.where(r_i // DH == c_i % 2, kv_v[p], 0.0).astype(BF16)
        return 3, _touch(z)

    def key_tasks(i, u, slot):
        return [P(phi_k, i, u, slot, q, t) for q in PAIRS for t in range(2)]

    def value_tasks(i, u, slot):
        return [P(v_round, i, u, slot, q) for q in PAIRS]

    sync(k_copies(0), x0_cps[:1])
    sync(k_copies(1), x0_cps[1:])
    run(ln_tasks(0))
    sync(k_copies(2), k_copies(0))
    prep_phi(0, UW)
    fold(1, 0)
    run(weight_tasks(1, 0))
    starts = [k_copies(3), [v_copy(0)], [v_copy(1), x1_cp], [v_copy(2)]]
    for u in range(NU):
        a = 2 if u else 3
        if u + 1 < NU:
            job = [P(sync, starts[u], k_copies(u + 1))] + ([] if u else [P(prep_phi, UW, D)]) + [P(fold, 1, u + 1)]
            late = weight_tasks(1, u + 1)
        else:
            job = [P(sync, starts[u], [v_copy(0)])]
            late = weight_tasks(2, 0)
        early = key_tasks(0, u - 1, 2 + (u - 1) % 2) if u else []
        proj(1, u, 0, 2 + u % 2, _join(_spread(early, 0, a + 1), _spread(late, a + 1)), {a: job})
    starts = [[v_copy(3)], [x23_cp], later_cps]
    waits = [[v_copy(1), x1_cp], [v_copy(2)], [v_copy(3)]]
    ln = ln_tasks(1)
    c0, c1 = len(ln) // 4, len(ln) // 2
    ln = _join(_spread(ln[:c0], 3, 7, 28), _spread(ln[c0:c1], 10, 14, 28), _spread(ln[c1:], 17, 25, 28))
    for u in range(NU):
        early = value_tasks(0, u - 1, (u - 1) % 2) if u else key_tasks(0, NU - 1, 3)
        jobs = {NPROD - 1: [P(kv_update, 0, u - 1)]} if u else {}
        plan = _spread(early)
        if u + 1 < NU:
            jobs[2] = [P(sync, starts[u], waits[u])]
            plan = _join(_spread(early, 0, 3), _spread(weight_tasks(2, u + 1), 3))
        proj(2, u, 0, u % 2, _join(plan, ln[NPROD * u:NPROD * (u + 1)]), jobs)

    wo_tasks = [P(wo_terms, u, g, ks) for u in range(NU) for g in range(NU) for ks in ((0, 1, 2), (3, 4, 5, 6))]
    prev = (0, NU - 1)
    for i in range(1, NTILE):
        if i == 1:
            sync([], [x23_cp])
        if i == 3:
            sync(ffn_cps, later_cps)
        side = ln_tasks(i + 1) + idle * 4 if i + 1 < NTILE else wo_tasks[2 * NU:]
        for u in range(NU):
            mine = side[u * len(side) // NU:(u + 1) * len(side) // NU]
            cut = len(mine) * 11 // 14 if i + 1 < NTILE else len(mine)
            k_tasks = _merge(value_tasks(*prev, 1), mine[:cut])
            v_tasks = _merge(key_tasks(i, u, 0), mine[cut:])
            k_jobs = {NPROD - 1: [P(kv_update, *prev)]}
            if 3 <= i < 3 + NU:
                if u == 0:
                    k_jobs[0] = [P(fold, 0, i - 3)]
                v_tasks = _merge(v_tasks, weight_tasks(0, i - 3)[3 * u:3 * u + 3])
                k_tasks = _merge(k_tasks, wo_tasks[2 * (i - 3) + u // 2:2 * (i - 3) + (u + 1) // 2])
            if i == NTILE - 1 and u > 1:
                k_tasks = _merge(k_tasks, [P(kv_finish, (u - 2) * 4 + q) for q in range(4)])
            proj(1, u, i, 0, _spread(k_tasks), k_jobs)
            proj(2, u, i, 1, _spread(v_tasks))
            prev = (i, u)

    best = jnp.max(jnp.max(best_v[...], axis=0), axis=0, keepdims=True)
    first = jnp.min(jnp.min(jnp.where(best_v[...] == best[None], bidx_v[...], S), axis=0), axis=0, keepdims=True)
    idx = jnp.where(first[0, 0] == S, 0, first[0, 0])
    route_gate = _bf16_round(jax.nn.sigmoid(jnp.where(first == S, jnp.nan, best)))[:, 0:1]
    fix_grp = jnp.where(idx >= S - T, 0, idx // 16)
    fix_rows = pl.ds(pl.multiple_of(fix_grp * 16, 16), 16)
    fix_cp = copy(fix_v, out_hbm.at[fix_rows], 5)

    def ffn_input(begun):
        xsel = _bf16_round(_layernorm(x_v[pl.ds(pl.multiple_of((idx // 8) * 8, 8), 8), :].astype(F32)))
        xsel_v[...] = xsel
        sfix_v[...] = jnp.zeros(sfix_v.shape, F32)
        return 5, _touch(xsel)

    def ffn_up(c, which, h):
        half = slice(h * HD, (h + 1) * HD)
        gu_v[c % 2, which, h] = _dot(xsel_v[:, half], (wg_v, wu_v)[which][half, c * 128:(c + 1) * 128])
        if which and h:
            g = gu_v[c % 2, 0, 0] + gu_v[c % 2, 0, 1]
            h_v[c % 2] = _bf16_round(g * jax.nn.sigmoid(g) * (gu_v[c % 2, 1, 0] + gu_v[c % 2, 1, 1]))

    def ffn_down(c, h):
        half = slice(h * HD, (h + 1) * HD)
        y = _dot(h_v[c % 2], wd_v[c * 128:(c + 1) * 128, half])
        if c:
            y = y + y_v[:, half]
        y_v[:, half] = y
        finish_within(3, _touch(y))

    ffn = []
    for c in range(FF // 128):
        ffn += [P(ffn_up, c, which, h) for which in range(2) for h in range(2)]
        ffn += [P(ffn_down, c - 1, h) for h in range(2)] if c else []
    ffn += [P(ffn_down, FF // 128 - 1, h) for h in range(2)]

    def routed_update(cols):
        y = y_v[:, cols]
        mine = lax.broadcasted_iota(jnp.int32, y.shape, 0) == idx % 8
        return _bf16_round(_bf16_round(jnp.sum(jnp.where(mine, y, 0.0), axis=0, keepdims=True)) * route_gate)

    def fix_routed():
        b = xn_v[fix_rows, :].astype(F32)
        row = lax.broadcasted_iota(jnp.int32, b.shape, 0) + fix_grp * 16
        b = jnp.where(row == idx, _bf16_round(b + routed_update(slice(None))), b)
        fix_v[...] = _gated(x_v[fix_rows, :].astype(F32), b, sfix_v[...]).astype(BF16)

    def phi_q(u, slot, q, t, begun):
        e_pos, e_neg, r_pos, r_neg = _dual_exp(pair_block(slot, q, t))
        a = jnp.sum(e_pos * z_v[u * 4 + q, :PR].reshape(8, 8, 128), axis=0)
        b = jnp.sum(e_neg * z_v[u * 4 + q, PR:].reshape(8, 8, 128), axis=0)
        r_den = _recip(_pair_reduce(r_pos * a + r_neg * b, jnp.add) + 1e-6)
        f = _features(e_pos, e_neg, r_pos * r_den, r_neg * r_den)
        return 5, _touch(keep_features(u, q, t, f))

    def attend(u):
        for q in PAIRS:
            o = _dot(kvt_v[u * 4 + q], pltpu.bitcast(phi_v[u][q, :T // 2], BF16), NT)
            for t in range(2):
                ot_v[q // 2, t, (q % 2) * PR:(q % 2 + 1) * PR, :] = o[:, t * 128:(t + 1) * 128]

    def o_terms(j, u, ks, begun):
        outs = [_transposed_words(_lhs_term(k, lambda t, g: ot_v[g, t])) for k in ks]
        for k, words in zip(ks, outs):
            os_v[j % 2][k, :, u * 128:(u + 1) * 128] = words
        return 2, _touch(*outs)

    def out_proj(j, u, slot, plan):
        products(slot, lambda k: os_v[j % 2][k], lambda k: pltpu.bitcast(wos_v[u, k], BF16), NN, plan, {})

    def epilogue(j, u, slot, t, c, begun):
        r0 = j * T + t * HT + c * 64
        cols = slice(u * UW, (u + 1) * UW)
        s = jnp.concatenate([block(slot, t, h, slice(c * 64, (c + 1) * 64)) for h in range(2)], axis=1)
        b = xn_v[r0:r0 + 64, cols].astype(F32)
        kept = []
        if j == NTILE - 1:
            row = lax.broadcasted_iota(jnp.int32, b.shape, 0) + r0
            b = jnp.where(row == idx, _bf16_round(b + routed_update(cols)), b)
        else:
            keep = sfix_v[:, cols]
            for g in range(4):
                keep = jnp.where(fix_grp == r0 // 16 + g, s[g * 16:(g + 1) * 16], keep)
            sfix_v[:, cols] = keep
            kept = [keep]
        res = _gated(x_v[r0:r0 + 64, cols].astype(F32), b, s)
        out_v[r0:r0 + 64, cols] = res.astype(BF16)
        return 2, _touch(res, *kept)

    steps = [(j, u) for j in range(NTILE) for u in range(NU)]
    lag = NU + 1
    waiting = []
    for n in range(len(steps) + lag + 1):
        cur = steps[n] if n < len(steps) else None
        att = steps[n - 1] if 1 <= n <= len(steps) else None
        out = steps[n - lag] if lag <= n < len(steps) + lag else None
        epi = steps[n - lag - 1] if n > lag else None
        ends = [P(epilogue, *epi, 2 + (n - 1) % 2, t, c) for t in (1, 0) for c in range(2)] if epi else []
        soft = [P(phi_q, cur[1], n % 2, q, t) for q in PAIRS for t in range(2)] if cur else []
        terms = [P(o_terms, *att, ks) for ks in ((0, 1), (2, 3, 4), (5, 6))] if att else []
        if n == 1:
            sync([], ffn_cps)
        if n == 0:
            plan = _join(_spread(value_tasks(*prev, 1), 0, 3), _spread([P(kv_finish, 8 + q) for q in range(4)], 3))
            proj(0, cur[1], cur[0], 0, plan, {5: [P(kv_update, *prev)]})
            waiting = [ffn_input] + soft
        elif not out and cur:
            proj(0, cur[1], cur[0], n % 2, _spread(waiting, 0, NPROD - 1))
            attend(att[1])
            waiting = _merge(terms, soft) + ([P(kv_finish, 12 + q) for q in range(4)] if n == 2 else [])
        elif cur:
            jobs = {k: [job] for k, job in enumerate(ffn[(n - lag) * NPROD:(n - lag + 1) * NPROD])}
            proj(0, cur[1], cur[0], n % 2, _join(_spread(waiting, 0, 5), _spread(ends)), jobs)
            waiting = []
            attend(att[1])
            if epi and epi[1] == NU - 1:
                out_copy(epi[0]).start()
            out_proj(*out, 2 + n % 2, _spread(terms + soft))
        elif out:
            if att:
                attend(att[1])
            out_proj(*out, 2 + n % 2, _spread(_merge(terms, ends)))
            if epi == (NTILE - 2, NU - 1):
                out_copy(epi[0]).start()
            if epi[0] == NTILE - 1:
                out_copy(*epi).start()
            if epi == (NTILE - 1, 0):
                sync([], [out_copy(j) for j in range(NTILE - 1)])
                fix_routed()
                fix_cp.start()
        else:
            for k, t in enumerate((1, 0)):
                run(ends[2 * k:2 * k + 2])
                out_copy(*epi, t).start()

    pins = [r for k, r in work.items() if k.rstrip('0123') in PINNED]
    pins = [copy(r.at[(0,) * (len(r.shape) - 2) + (pl.ds(0, 8), pl.ds(0, 128))], work[r.dtype.name].at[k], 5)
            for k, r in enumerate(pins)]
    sync(pins, pins + [fix_cp] + [out_copy(NTILE - 1, u) for u in range(NU - 1)]
         + [out_copy(NTILE - 1, NU - 1, t) for t in range(2)])


@jax.jit
def pallas_recurrent_scan__linear_kernel_hedgehog__moe_arch_mod__prompt_kernel(
        A_x, A_wqkv, A_w_phi, A_wo, B_x, B_w_r, B_w_gate, B_w_up, B_w_down):
    del B_x
    work = dict(
        order=((1, NORDER, 8, 128), U32), float32=((16, 8, 128), F32), uint32=((16, 8, 128), U32),
        bfloat16=((16, 8, 128), BF16),
        bd=((128, D), BF16), fold=((NU, 2, 128, D), F32), wt=((3, NU, NPROD, 64, HD), U32),
        xn=((S, D), BF16), score=((S // 8, 8, 128), F32),
        best=((NTILE, 8, 128), F32), bidx=((NTILE, 8, 128), jnp.int32),
        kv=((H // 2, PR, 128), F32), kvt=((H // 2, PR, 128), BF16), z=((H // 2, 128, 128), F32),
        vt=((NU, 4, PR, 2 * T), BF16), ot=((2, 2, 128, 128), F32),
        xsel=((8, D), F32), gu=((2, 2, 2, 8, 128), F32), h=((2, 8, 128), F32), y=((8, D), F32), sfix=((16, D), F32))
    work.update({'m%d' % k: ((NPROD, 128, 128), F32) for k in range(4)})
    work.update({'phi%d' % k: ((4, T, 128), U32) for k in range(NU)})
    work.update(xs=((NTILE, NPROD, HT, HD), BF16), wos=((NU, NPROD, HD // 2, 128), U32))
    work.update({'os%d' % k: ((NPROD, HT // 2, HD), U32) for k in range(2)})
    hbm = pl.BlockSpec(memory_space=pl.ANY)
    out = pl.pallas_call(
        _kernel,
        in_specs=[hbm] * 8,
        out_specs=hbm,
        out_shape=jax.ShapeDtypeStruct((S, D), BF16),
        scratch_shapes=[
            pltpu.VMEM((S, D), BF16),
            pltpu.VMEM((D, 3 * D), BF16),
            pltpu.VMEM((D, DH), BF16),
            pltpu.VMEM((8, 128), BF16),
            pltpu.VMEM((D, D), BF16),
            pltpu.VMEM((D, FF), BF16),
            pltpu.VMEM((D, FF), BF16),
            pltpu.VMEM((FF, D), BF16),
            pltpu.VMEM((S, D), BF16),
            pltpu.VMEM((16, D), BF16),
            {k: pltpu.VMEM(shape, dt) for k, (shape, dt) in work.items()},
            pltpu.SemaphoreType.DMA((6,)),
        ],
        compiler_params=pltpu.CompilerParams(vmem_limit_bytes=110 * 2**20),
    )(A_x.reshape(S, D), A_wqkv, A_w_phi.reshape(D, DH), A_wo, B_w_r.reshape(8, 128),
      B_w_gate, B_w_up, B_w_down)
    return out.reshape(1, S, D)
```
